```python
import jax
import jax.numpy as jnp

def _softmax(x, axis=-1):
    return jax.nn.softmax(x, axis=axis)
def _gelu(x):
    return jax.nn.gelu(x, approximate=True)
def _silu(x):
    return jax.nn.silu(x)
def _sigmoid(x):
    return jax.nn.sigmoid(x)
def _layernorm(x, axis=-1, eps=1e-5):
    m = jnp.mean(x, axis=axis, keepdims=True)
    v = jnp.var(x, axis=axis, keepdims=True)
    return (x - m) / jnp.sqrt(v + eps)
def _scatter_add(tgt, idx, src, axis=0):
    return tgt.at[idx].add(src)
def _segment_sum(src, seg, n):
    return jax.ops.segment_sum(src, seg, n)
class _Rng:
    def __init__(self, key):
        self._k = key
    def _next(self):
        self._k, sub = jax.random.split(self._k)
        return sub
    def normal(self, shape):
        return jax.random.normal(self._next(), shape, dtype=jnp.bfloat16)
    def randint(self, lo, hi, shape):
        return jax.random.randint(self._next(), shape, lo, hi, dtype=jnp.int32)
    def uniform(self, shape, lo=0.0, hi=1.0):
        return jax.random.uniform(self._next(), shape, jnp.bfloat16, lo, hi)
    def permutation(self, n):
        return jax.random.permutation(self._next(), n)


kernel_name = 'sequential_preLN__sliding_local_dilated__glu_gated_geglu__prompt'

def setup_inputs():
    _rng = _Rng(jax.random.key(int.from_bytes(__import__("os").urandom(4), "little")))
    _w = (lambda a: (lambda t: t.astype(jnp.bfloat16) if jnp.issubdtype(t.dtype, jnp.floating) else t)(jnp.asarray(a)))
    def _A_setup():
        B, S, D = 1, 2048, 1024
        return {
            "x": _w((lambda *s: _rng.normal(s) * 0.05)(B, S, D)),
            "wqkv": _w((lambda *s: _rng.normal(s) * 0.05)(D, 3 * D)),
            "wo": _w((lambda *s: _rng.normal(s) * 0.05)(D, D)),
        }
    _A_in = _A_setup()

    def _B_setup():
        B, S, Dm, Df = 1, 2048, 1024, 3584
        return {
            "x": _w((lambda *s: _rng.normal(s) * 0.05)(B, S, Dm)),
            "w_gate": _w((lambda *s: _rng.normal(s) * 0.05)(Dm, Df) * (Dm ** -0.5)),
            "w_up": _w((lambda *s: _rng.normal(s) * 0.05)(Dm, Df) * (Dm ** -0.5)),
            "w_down": _w((lambda *s: _rng.normal(s) * 0.05)(Df, Dm) * (Df ** -0.5)),
        }
    _B_in = _B_setup()

    return {
        "A_x": _A_in["x"],
        "A_wqkv": _A_in["wqkv"],
        "A_wo": _A_in["wo"],
        "B_x": _B_in["x"],
        "B_w_gate": _B_in["w_gate"],
        "B_w_up": _B_in["w_up"],
        "B_w_down": _B_in["w_down"],
    }

def reference(A_x, A_wqkv, A_wo, B_x, B_w_gate, B_w_up, B_w_down):
    def _A_ref(x, wqkv, wo):
        B, S, D = x.shape
        H = 32; Dh = D // H
        W, dil = 8, 2
        qkv = (lambda x, *d: x.transpose(*d))((x @ wqkv).reshape(B, S, 3, H, Dh), 2, 0, 3, 1, 4)
        q, k, v = qkv[0], qkv[1], qkv[2]
        scale = Dh ** -0.5
        pos = jnp.arange(S)
        off = jnp.arange(W) * dil
        idx = pos[:, None] - off[None, :]
        mask = idx >= 0
        idx_c = jnp.where(mask, idx, 0).reshape(-1)
        kg = k[:, :, idx_c, :].reshape(B, H, S, W, Dh)
        vg = v[:, :, idx_c, :].reshape(B, H, S, W, Dh)
        logits = jnp.einsum("bhsd,bhswd->bhsw", q, kg) * scale
        logits = jnp.where(mask[None, None, :, :], logits, -1e9)
        attn = _softmax(logits, axis=-1)
        o = jnp.einsum("bhsw,bhswd->bhsd", attn, vg)
        return (lambda x, *d: x.transpose(*d))(o, 0, 2, 1, 3).reshape(B, S, D) @ wo

    def _B_ref(x, w_gate, w_up, w_down):
        g = jnp.einsum("bsd,df->bsf", x, w_gate)
        u = jnp.einsum("bsd,df->bsf", x, w_up)
        h = _gelu(g) * u
        return jnp.einsum("bsf,fd->bsd", h, w_down)

    x = A_x
    h = x + _A_ref(_layernorm(x, axis=-1), A_wqkv, A_wo)
    h2 = h + _B_ref(_layernorm(h, axis=-1), B_w_gate, B_w_up, B_w_down)
    return h2
```

```python
import jax
import jax.numpy as jnp
import numpy as np
import jax.experimental.pallas as pl
import jax.experimental.pallas.tpu as pltpu

S, D, F = 2048, 1024, 3584
NB = D // 128
W, DIL, HALO = 8, 2, 16
T1, T2, T3 = 512, 512, 512
FC = 512
R = 16
EPS = 1e-5
SCALE = 32 ** -0.5
f32, bf16 = jnp.float32, jnp.bfloat16


def _dot(a, b):
    return jnp.dot(a, b, preferred_element_type=f32)


def _layernorm(x):
    m = jnp.mean(x, axis=-1, keepdims=True)
    c = x - m
    v = jnp.mean(c * c, axis=-1, keepdims=True)
    return c * jax.lax.rsqrt(v + EPS)


def _swap_bits(blocks, axis, bits):
    n = blocks[0].shape[axis]
    idx = jax.lax.broadcasted_iota(jnp.int32, blocks[0].shape, axis)
    for t, b in enumerate(bits):
        hi = (idx & (1 << b)) != 0
        new = list(blocks)
        for j0 in range(len(blocks)):
            if j0 & (1 << t):
                continue
            j1 = j0 | (1 << t)
            new[j0] = jnp.where(hi, pltpu.roll(blocks[j1], 1 << b, axis), blocks[j0])
            new[j1] = jnp.where(hi, blocks[j1], pltpu.roll(blocks[j0], n - (1 << b), axis))
        blocks = new
    return blocks


def _permute_cols(w_ref, r0, nr, c0):
    blocks = [pltpu.bitcast(w_ref[pl.ds(r0, nr), c0 + 128 * j:c0 + 128 * (j + 1)], jnp.int32) for j in range(NB)]
    for j, blk in enumerate(_swap_bits(blocks, 1, (1, 2, 3))):
        w_ref[pl.ds(r0, nr), c0 + 128 * j:c0 + 128 * (j + 1)] = pltpu.bitcast(blk, bf16)


def _permute_rows(w_ref, m):
    blocks = [pltpu.bitcast(w_ref[pl.ds(128 * j + m * 16, 16), :], jnp.int32) for j in range(NB)]
    for j, blk in enumerate(_swap_bits(blocks, 0, (0, 1, 2))):
        w_ref[pl.ds(128 * j + m * 16, 16), :] = pltpu.bitcast(blk, bf16)


def _attend(q_ref, k_ref, v_ref, o_ref, r0, ro, masked):
    lane = jax.lax.broadcasted_iota(jnp.int32, (R, 128), 1)
    q = [q_ref[j, pl.ds(r0, R), :] for j in range(NB)]
    logits = []
    for w in range(W):
        s = None
        for j in range(NB):
            t = q[j] * k_ref[j, pl.ds(r0 + HALO - DIL * w, R), :]
            s = t if s is None else s + t
        for b in (1, 16):
            s = s + jnp.where((lane & b) != 0, pltpu.roll(s, b, 1), pltpu.roll(s, 128 - b, 1))
        s = s * SCALE
        if masked and w:
            pos = r0 + jax.lax.broadcasted_iota(jnp.int32, (R, 128), 0)
            s = jnp.where(pos >= DIL * w, s, -1e9)
        logits.append(s)
    m = logits[0]
    for s in logits[1:]:
        m = jnp.maximum(m, s)
    e = [jnp.exp(s - m) for s in logits]
    den = e[0]
    for t in e[1:]:
        den = den + t
    inv = 1.0 / den
    p = [t * inv for t in e]
    for j in range(NB):
        o = None
        for w in range(W):
            t = p[w] * v_ref[j, pl.ds(r0 + HALO - DIL * w, R), :]
            o = t if o is None else o + t
        o_ref[pl.ds(ro, R), 128 * j:128 * (j + 1)] = o.astype(bf16)


def _kernel(x_hbm, wqkv_hbm, wo_hbm, wg_hbm, wu_hbm, wd_hbm, out_hbm,
            x_v, wqkv_v, wo_v, wg_v, wu_v, wd_v, q_v, k_v, v_v, o_v, h_v, hn_v, out_v, sems, osem):
    cps = [pltpu.make_async_copy(s, d, sems.at[i]) for i, (s, d) in enumerate(
        [(wqkv_hbm, wqkv_v), (x_hbm, x_v), (wo_hbm, wo_v), (wg_hbm, wg_v), (wu_hbm, wu_v), (wd_hbm, wd_v)])]
    for c in cps[:3]:
        c.start()
    with jax.named_scope("sc_0_wait"):
        cps[0].wait()
    for c in cps[3:]:
        c.start()

    with jax.named_scope("sc_1_perm"):
        @pl.loop(0, D // 32)
        def _(i):
            for c in range(3):
                _permute_cols(wqkv_v, pl.multiple_of(i * 32, 32), 32, c * D)
    cps[1].wait()
    cps[2].wait()
    with jax.named_scope("sc_2_permo"):
        for m in range(8):
            _permute_rows(wo_v, m)

    with jax.named_scope("sc_3_qkv"):
        @pl.loop(0, S // T1)
        def _(i):
            r0 = pl.multiple_of(i * T1, T1)
            xn = _layernorm(x_v[pl.ds(r0, T1), :].astype(f32)).astype(bf16)
            for c, (ref, off) in enumerate(((q_v, 0), (k_v, HALO), (v_v, HALO))):
                y = _dot(xn, wqkv_v[:, c * D:(c + 1) * D])
                for j in range(NB):
                    ref[j, pl.ds(r0 + off, T1), :] = y[:, 128 * j:128 * (j + 1)]

    for ref in (k_v, v_v):
        for j in range(NB):
            ref[j, 0:HALO, :] = jnp.broadcast_to(ref[j, HALO:HALO + 1, :], (HALO, 128))

    with jax.named_scope("sc_4_attn"):
        @pl.loop(0, S // T2)
        def _(i):
            r0 = pl.multiple_of(i * T2, T2)
            for c in range(T2 // R):
                _attend(q_v, k_v, v_v, o_v, r0 + c * R, c * R, c * R < HALO)
            h = x_v[pl.ds(r0, T2), :].astype(f32) + _dot(o_v[...], wo_v[...])
            h_v[pl.ds(r0, T2), :] = h
            hn_v[pl.ds(r0, T2), :] = _layernorm(h).astype(bf16)

    for c in cps[3:]:
        c.wait()

    def out_copy(i):
        r0 = pl.multiple_of(i * T3, T3)
        return pltpu.make_async_copy(out_v.at[pl.ds(r0, T3), :], out_hbm.at[pl.ds(r0, T3), :], osem.at[i])

    with jax.named_scope("sc_5_ffn"):
        @pl.loop(0, S // T3)
        def _(i):
            r0 = pl.multiple_of(i * T3, T3)
            hn = hn_v[pl.ds(r0, T3), :]
            acc = h_v[pl.ds(r0, T3), :]
            for c in range(F // FC):
                g = _dot(hn, wg_v[:, c * FC:(c + 1) * FC])
                u = _dot(hn, wu_v[:, c * FC:(c + 1) * FC])
                a = (jax.nn.gelu(g, approximate=True) * u).astype(bf16)
                acc = acc + _dot(a, wd_v[c * FC:(c + 1) * FC, :])
            out_v[pl.ds(r0, T3), :] = acc.astype(bf16)
            out_copy(i).start()

    with jax.named_scope("sc_6_out"):
        for i in range(S // T3):
            out_copy(i).wait()


@jax.jit
def pallas_sequential_preLN__sliding_local_dilated__glu_gated_geglu__prompt_kernel(
        A_x, A_wqkv, A_wo, B_x, B_w_gate, B_w_up, B_w_down):
    del B_x
    any_spec = pl.BlockSpec(memory_space=pl.ANY)
    out = pl.pallas_call(
        _kernel,
        in_specs=[any_spec] * 6,
        out_specs=any_spec,
        out_shape=jax.ShapeDtypeStruct((S, D), bf16),
        scratch_shapes=[
            pltpu.VMEM((S, D), bf16), pltpu.VMEM((D, 3 * D), bf16), pltpu.VMEM((D, D), bf16),
            pltpu.VMEM((D, F), bf16), pltpu.VMEM((D, F), bf16), pltpu.VMEM((F, D), bf16),
            pltpu.VMEM((NB, S, 128), f32), pltpu.VMEM((NB, S + HALO, 128), f32), pltpu.VMEM((NB, S + HALO, 128), f32),
            pltpu.VMEM((T2, D), bf16), pltpu.VMEM((S, D), f32), pltpu.VMEM((S, D), bf16), pltpu.VMEM((S, D), bf16),
            pltpu.SemaphoreType.DMA((6,)), pltpu.SemaphoreType.DMA((S // T3,)),
        ],
        compiler_params=pltpu.CompilerParams(vmem_limit_bytes=120 * 1024 * 1024),
    )(A_x.reshape(S, D), A_wqkv, A_wo, B_w_gate, B_w_up, B_w_down)
    return out.reshape(1, S, D)
```

```python
import jax
import jax.numpy as jnp
import numpy as np
import jax.experimental.pallas as pl
import jax.experimental.pallas.tpu as pltpu

S, D, F = 2048, 1024, 3584
NB = D // 128
W, DIL, HALO = 8, 2, 16
T1, T2, T3 = 256, 128, 256
NH = 2
FC = 512
R = 16
EPS = 1e-5
SCALE = 32 ** -0.5
f32, bf16 = jnp.float32, jnp.bfloat16


def _dot(a, b):
    return jnp.dot(a, b, preferred_element_type=f32)


def _layernorm(x):
    m = jnp.mean(x, axis=-1, keepdims=True)
    c = x - m
    v = jnp.mean(c * c, axis=-1, keepdims=True)
    return c * jax.lax.rsqrt(v + EPS)


def _swap_bits(blocks, axis, bits):
    n = blocks[0].shape[axis]
    idx = jax.lax.broadcasted_iota(jnp.int32, blocks[0].shape, axis)
    for t, b in enumerate(bits):
        hi = (idx & (1 << b)) != 0
        new = list(blocks)
        for j0 in range(len(blocks)):
            if j0 & (1 << t):
                continue
            j1 = j0 | (1 << t)
            new[j0] = jnp.where(hi, pltpu.roll(blocks[j1], 1 << b, axis), blocks[j0])
            new[j1] = jnp.where(hi, blocks[j1], pltpu.roll(blocks[j0], n - (1 << b), axis))
        blocks = new
    return blocks


def _permute_cols(w_ref, r0, nr, c0):
    blocks = [pltpu.bitcast(w_ref[pl.ds(r0, nr), c0 + 128 * j:c0 + 128 * (j + 1)], jnp.int32) for j in range(NB)]
    for j, blk in enumerate(_swap_bits(blocks, 1, (1, 2, 3))):
        w_ref[pl.ds(r0, nr), c0 + 128 * j:c0 + 128 * (j + 1)] = pltpu.bitcast(blk, bf16)


def _permute_rows(w_ref, m):
    blocks = [pltpu.bitcast(w_ref[pl.ds(128 * j + m * 16, 16), :], jnp.int32) for j in range(NB)]
    for j, blk in enumerate(_swap_bits(blocks, 0, (0, 1, 2))):
        w_ref[pl.ds(128 * j + m * 16, 16), :] = pltpu.bitcast(blk, bf16)


def _attend(q_ref, k_ref, v_ref, o_ref, kr, r, pos0):
    lane = jax.lax.broadcasted_iota(jnp.int32, (R, 128), 1)
    q = [q_ref[j, r:r + R, :] for j in range(NB)]
    logits = []
    for w in range(W):
        s = None
        for j in range(NB):
            t = q[j] * k_ref[j, pl.ds(kr + HALO - DIL * w, R), :]
            s = t if s is None else s + t
        for b in (1, 16):
            s = s + jnp.where((lane & b) != 0, pltpu.roll(s, b, 1), pltpu.roll(s, 128 - b, 1))
        s = s * SCALE
        if pos0 is not None and w:
            pos = pos0 + jax.lax.broadcasted_iota(jnp.int32, (R, 128), 0)
            s = jnp.where(pos >= DIL * w, s, -1e9)
        logits.append(s)
    m = logits[0]
    for s in logits[1:]:
        m = jnp.maximum(m, s)
    e = [jnp.exp(s - m) for s in logits]
    den = e[0]
    for t in e[1:]:
        den = den + t
    inv = 1.0 / den
    p = [t * inv for t in e]
    for j in range(NB):
        o = None
        for w in range(W):
            r0 = r + HALO - DIL * w
            t = p[w] * v_ref[j, r0:r0 + R, :]
            o = t if o is None else o + t
        o_ref[r:r + R, 128 * j:128 * (j + 1)] = o.astype(bf16)


def _kernel(x_hbm, wqkv_hbm, wo_hbm, wg_hbm, wu_hbm, wd_hbm, out_hbm,
            x_v, xn_v, wq_v, wk_v, wv_v, wo_v, wg_v, wu_v, wd_v, q_v, k_v, v_v, o_v, h_v, hn_v, out_v,
            xsem, wsem, fsem, osem):
    n1 = S // T1
    slab = D // n1

    def rows(i, n):
        return pl.ds(pl.multiple_of(i * n, n), n)

    def x_copy(i):
        return pltpu.make_async_copy(x_hbm.at[rows(i, T1), :], x_v.at[rows(i, T1), :], xsem.at[i])

    def w_copy(c, i):
        dst = (wq_v, wk_v, wv_v)[c]
        return pltpu.make_async_copy(wqkv_hbm.at[rows(i, slab), c * D:(c + 1) * D], dst.at[rows(i, slab), :],
                                     wsem.at[c * n1 + i])

    f_copies = [pltpu.make_async_copy(s, d, fsem.at[i]) for i, (s, d) in enumerate(
        [(wo_hbm, wo_v), (wg_hbm, wg_v), (wu_hbm, wu_v), (wd_hbm, wd_v)])]

    def out_copy(i):
        return pltpu.make_async_copy(out_v.at[rows(i, T3), :], out_hbm.at[rows(i, T3), :], osem.at[i])

    for i in range(n1):
        w_copy(1, i).start()
        if i == 1:
            x_copy(0).start()
    x_copy(1).start()
    w_copy(0, 0).start()
    w_copy(2, 0).start()

    with jax.named_scope("sc_0_permk"):
        @pl.loop(0, n1)
        def _(i):
            w_copy(1, i).wait()
            _permute_cols(wk_v, pl.multiple_of(i * slab, slab), slab, 0)

    def ln1(i):
        xn_v[rows(i, T1), :] = _layernorm(x_v[rows(i, T1), :].astype(f32)).astype(bf16)

    with jax.named_scope("sc_1_ln"):
        x_copy(0).wait()
        ln1(0)

    with jax.named_scope("sc_2_k"):
        @pl.loop(0, n1)
        def _(i):
            @pl.when(i + 2 < n1)
            def _():
                x_copy(i + 2).start()

            @pl.when(i + 1 < n1)
            def _():
                w_copy(0, i + 1).start()
                w_copy(2, i + 1).start()
                x_copy(i + 1).wait()

            @pl.when(i == n1 - 2)
            def _():
                f_copies[0].start()
            w_copy(0, i).wait()
            w_copy(2, i).wait()
            y = _dot(xn_v[rows(i, T1), :], wk_v[...])
            for j in range(NB):
                k_v[j, pl.ds(pl.multiple_of(i * T1, T1) + HALO, T1), :] = y[:, 128 * j:128 * (j + 1)]
            ln1(jnp.minimum(i + 1, n1 - 1))
            _permute_cols(wq_v, pl.multiple_of(i * slab, slab), slab, 0)
            _permute_cols(wv_v, pl.multiple_of(i * slab, slab), slab, 0)

    with jax.named_scope("sc_3_permo"):
        f_copies[0].wait()
        for c in f_copies[1:]:
            c.start()
        for m in range(8):
            _permute_rows(wo_v, m)
        for j in range(NB):
            k_v[j, 0:HALO, :] = jnp.broadcast_to(k_v[j, HALO:HALO + 1, :], (HALO, 128))
            v_v[j, NH * T2:NH * T2 + HALO, :] = jnp.zeros((HALO, 128), f32)

    with jax.named_scope("sc_4_attn"):
        @pl.loop(0, S // (NH * T2))
        def _(i):
            r0 = pl.multiple_of(i * (NH * T2), NH * T2)
            prev = [v_v[j, NH * T2:NH * T2 + HALO, :] for j in range(NB)]

            def qv(a):
                xn = xn_v[pl.ds(r0 + a * T2, T2), :]
                y = _dot(xn, wq_v[...])
                for j in range(NB):
                    q_v[j, a * T2:(a + 1) * T2, :] = y[:, 128 * j:128 * (j + 1)]
                y = _dot(xn, wv_v[...])
                for j in range(NB):
                    yj = y[:, 128 * j:128 * (j + 1)]
                    v_v[j, HALO + a * T2:HALO + (a + 1) * T2, :] = yj
                    if a == 0:
                        v_v[j, 0:HALO, :] = jnp.where(i > 0, prev[j], jnp.broadcast_to(yj[0:1, :], (HALO, 128)))

            def attn(a):
                for c in range(a * T2, (a + 1) * T2, R):
                    _attend(q_v, k_v, v_v, o_v, r0 + c, c, r0 + c if c < HALO else None)

            def proj(a):
                rr = pl.ds(r0 + a * T2, T2)
                h_v[rr, :] = x_v[rr, :].astype(f32) + _dot(o_v[a * T2:(a + 1) * T2, :], wo_v[...])

            qv(0)
            for a in range(NH):
                if a + 1 < NH:
                    qv(a + 1)
                if a > 0:
                    proj(a - 1)
                attn(a)
            proj(NH - 1)

    with jax.named_scope("sc_5_ln"):
        for c in f_copies[1:]:
            c.wait()
        hn_v[...] = _layernorm(h_v[0:T3, :]).astype(bf16)

    with jax.named_scope("sc_6_ffn"):
        @pl.loop(0, S // T3)
        def _(i):
            hn = hn_v[...]
            acc = h_v[rows(i, T3), :]
            for c in range(F // FC):
                g = _dot(hn, wg_v[:, c * FC:(c + 1) * FC])
                u = _dot(hn, wu_v[:, c * FC:(c + 1) * FC])
                a = (jax.nn.gelu(g, approximate=True) * u).astype(bf16)
                if c == F // FC - 1:
                    hn_v[...] = _layernorm(h_v[rows(jnp.minimum(i + 1, S // T3 - 1), T3), :]).astype(bf16)
                acc = acc + _dot(a, wd_v[c * FC:(c + 1) * FC, :])
            out_v[rows(i, T3), :] = acc.astype(bf16)
            out_copy(i).start()

    with jax.named_scope("sc_7_out"):
        for i in range(S // T3):
            out_copy(i).wait()


@jax.jit
def pallas_sequential_preLN__sliding_local_dilated__glu_gated_geglu__prompt_kernel(
        A_x, A_wqkv, A_wo, B_x, B_w_gate, B_w_up, B_w_down):
    del B_x
    any_spec = pl.BlockSpec(memory_space=pl.ANY)
    out = pl.pallas_call(
        _kernel,
        in_specs=[any_spec] * 6,
        out_specs=any_spec,
        out_shape=jax.ShapeDtypeStruct((S, D), bf16),
        scratch_shapes=[
            pltpu.VMEM((S, D), bf16), pltpu.VMEM((S, D), bf16),
            pltpu.VMEM((D, D), bf16), pltpu.VMEM((D, D), bf16), pltpu.VMEM((D, D), bf16), pltpu.VMEM((D, D), bf16),
            pltpu.VMEM((D, F), bf16), pltpu.VMEM((D, F), bf16), pltpu.VMEM((F, D), bf16),
            pltpu.VMEM((NB, NH * T2, 128), f32), pltpu.VMEM((NB, S + HALO, 128), f32),
            pltpu.VMEM((NB, NH * T2 + HALO, 128), f32),
            pltpu.VMEM((NH * T2, D), bf16), pltpu.VMEM((S, D), f32), pltpu.VMEM((T3, D), bf16),
            pltpu.VMEM((S, D), bf16),
            pltpu.SemaphoreType.DMA((S // T1,)), pltpu.SemaphoreType.DMA((3 * S // T1,)),
            pltpu.SemaphoreType.DMA((4,)), pltpu.SemaphoreType.DMA((S // T3,)),
        ],
        compiler_params=pltpu.CompilerParams(vmem_limit_bytes=120 * 1024 * 1024),
    )(A_x.reshape(S, D), A_wqkv, A_wo, B_w_gate, B_w_up, B_w_down)
    return out.reshape(1, S, D)
```

```python
import jax
import jax.numpy as jnp
import jax.experimental.pallas as pl
import jax.experimental.pallas.tpu as pltpu

S, D, F = 2048, 1024, 3584
HEAD_DIM, WINDOW, DILATION = 32, 8, 2
EPS = 1e-5
NB = D // 128
HALO = 16
T = 256
M = T // 2
NT = S // T
NH = 2
R = 16
FC = 256
OK = OV = OQ = OO = OG = OD = '1304265'
NS = 1
LP = 1
JOIN = 1
FS = 3
FLAGS = None
ORDER = 'v0 q0 v1 q1 a0 a1 o0 o1'
TREE = 0
OPQ = (0, 0)
FFN = 1
PC = 512
NOCHK = True
NK = 4
f32, bf16, i32 = jnp.float32, jnp.bfloat16, jnp.int32

QUADRANTS = ((0, 0), (0, 1), (1, 0), (1, 1))


def _words(x):
    return pltpu.bitcast(x.astype(bf16), i32)


def _dot(a, b):
    return jnp.dot(pltpu.bitcast(a, bf16), pltpu.bitcast(b, bf16), preferred_element_type=f32)


def _layernorm(x):
    c = x - jnp.mean(x, axis=-1, keepdims=True)
    return c * jax.lax.rsqrt(jnp.mean(c * c, axis=-1, keepdims=True) + EPS)


def _lane_xor(x, bits):
    lane = jax.lax.broadcasted_iota(jnp.int32, x.shape, 1)
    return jnp.take_along_axis(x, lane ^ bits, axis=1, mode="promise_in_bounds")


def _exchange_lanes(blocks):
    lane = jax.lax.broadcasted_iota(jnp.int32, blocks[0].shape, 1)
    blocks = [_lane_xor(b, 2 * j) if j else b for j, b in enumerate(blocks)]
    for t in (1, 2, 4):
        hi = (lane & (2 * t)) != 0
        blocks = [jnp.where(hi, blocks[j ^ t], blocks[j]) for j in range(NB)]
    return [_lane_xor(b, 2 * j) if j else b for j, b in enumerate(blocks)]


def _exchange_rows(blocks):
    row = jax.lax.broadcasted_iota(jnp.int32, blocks[0].shape, 0)
    for t in (1, 2, 4):
        hi = (row & t) != 0
        blocks = [jnp.where(hi, blocks[j], pltpu.roll(blocks[j ^ t], 8 - t, 0)) if j & t else
                  jnp.where(hi, pltpu.roll(blocks[j ^ t], t, 0), blocks[j]) for j in range(NB)]
    return blocks


def _rhs_terms(b11, b12, b21, b22):
    c11, c12, c21, c22 = (b.astype(f32) for b in (b11, b12, b21, b22))
    return [_words(t) for t in (c11 + c22, b11, c12 - c22, c21 - c11, b22, c11 + c12, c21 + c22)]


def _lhs_terms(a11, a12, a21, a22):
    return [_words(t) for t in (a11 + a22, a21 + a22, a11, a22, a11 + a12, a21 - a11, a12 - a22)]


BLOCKS = (((0, 1), (3, 1), (4, -1), (6, 1)), ((2, 1), (4, 1)), ((1, 1), (3, 1)), ((0, 1), (1, -1), (2, 1), (5, 1)))


def _strassen(lhs, rhs, order):
    out = [None] * 4
    for i in map(int, order):
        m = _dot(lhs(i), rhs(i))
        for q, block in enumerate(BLOCKS):
            sign = dict(block).get(i)
            if sign is None:
                continue
            if out[q] is None:
                out[q] = (m, sign)
            else:
                acc, s = out[q]
                out[q] = (acc + m, s) if s == sign else (acc - m, 1) if s > 0 else (m - acc, 1)
    return [acc for acc, _ in out]


def _prepare_qkv(pairs, r, n):
    hb, k = NB // 2, n // 2
    blocks = _exchange_lanes([
        jnp.concatenate([_words(raw[a, pl.ds(r, n), 128 * j:128 * (j + 1)]) for raw, _ in pairs for a in (0, 1)])
        for j in range(NB)])
    for p, (_, w_ref) in enumerate(pairs):
        for j in range(hb):
            quads = [pltpu.bitcast(blocks[j + b * hb][(2 * p + a) * k:(2 * p + a + 1) * k], bf16)
                     for a, b in QUADRANTS]
            for i, t in enumerate(_rhs_terms(*quads)):
                w_ref[i, pl.ds(pl.multiple_of(r // 2, 8), k), 128 * j:128 * (j + 1)] = t


def _prepare_wo(raw, w_ref, m):
    hb = NB // 2
    for c in range(0, D // 2, 128):
        halves = []
        for c0 in (c, D // 2 + c):
            blocks = [_words(raw[j, pl.ds(pl.multiple_of(16 * m, 16), 16), c0:c0 + 128]) for j in range(NB)]
            halves.append([pltpu.bitcast(t, bf16) for t in _exchange_rows(blocks)])
        for j in range(hb):
            for i, t in enumerate(_rhs_terms(halves[0][j], halves[1][j], halves[0][j + hb], halves[1][j + hb])):
                w_ref[i, pl.ds(pl.multiple_of(64 * j + 8 * m, 8), 8), c:c + 128] = t


def _prepare_ffn(w_ref, r, c, n):
    nr = w_ref.shape[0] // 7
    at = lambda i: (pl.ds(i * nr + r, 16), slice(c, c + n))
    terms = _rhs_terms(*(w_ref[at(i)] for i in (1, 2, 3, 4)))
    for i in (0, 2, 3, 5, 6):
        w_ref[at(i)] = pltpu.bitcast(terms[i], bf16)


def _sum(t):
    if not TREE:
        acc = t[0]
        for a in t[1:]:
            acc = acc + a
        return acc
    while len(t) > 1:
        t = [a + b for a, b in zip(t[::2], t[1::2])]
    return t[0]


def _softmax(sums, pos):
    logits = []
    for w, s in enumerate(sums):
        for b in (1, 16):
            s = s + _lane_xor(s, b)
        s = s * HEAD_DIM ** -0.5
        if pos is not None and w:
            s = jnp.where(pos + jax.lax.broadcasted_iota(i32, s.shape, 0) >= DILATION * w, s, -1e9)
        logits.append(s)
    top = logits[0]
    for s in logits[1:]:
        top = jnp.maximum(top, s)
    e = [jnp.exp(s - top) for s in logits]
    den = e[0]
    for t in e[1:]:
        den = den + t
    inv = 1.0 / den
    return [t * inv for t in e]


def _attend(q_ref, k_ref, v_ref, r, kr, vr, pos):
    window = lambda ref, j, r0, w: ref[j, pl.ds(r0 + HALO - DILATION * w, R), :]
    q = [q_ref[j, r:r + R, :] for j in range(NB)]
    p = _softmax([_sum([q[j] * window(k_ref, j, kr, w) for j in range(NB)]) for w in range(WINDOW)], pos)
    return [_sum([p[w] * window(v_ref, j, vr, w) for w in range(WINDOW)]) for j in range(NB)]


def _kernel(x_hbm, wqkv_hbm, wo_hbm, wg_hbm, wu_hbm, wd_hbm, out_hbm,
            x_v, raw_v, n_v, wq_v, wk_v, wv_v, wo_v, q_v, k_v, v_v, o_v, h_v, act_v,
            xsem, wsem, osem):
    hb = NB // 2
    na = NT // NH
    out_v = x_v
    slab = D // 2 // NT

    def rows(i, n):
        return pl.ds(pl.multiple_of(i * n, n), n)

    def x_copy(i):
        return pltpu.make_async_copy(x_hbm.at[rows(i, T), :], x_v.at[rows(i, T), :], xsem.at[i])

    def out_copy(i):
        return pltpu.make_async_copy(out_v.at[rows(i, T), :], out_hbm.at[rows(i, T), :], osem)

    weights = ((wqkv_hbm, 0, NT), (wqkv_hbm, D, NK), (wqkv_hbm, 2 * D, NT),
               (wo_hbm, 0, NT), (wg_hbm, 0, na), (wu_hbm, 0, na), (wd_hbm, 0, na))

    def w_copies(which, i):
        src, c0, parts = weights[which]
        raw = raw_v[which]
        if which == 3:
            return [pltpu.make_async_copy(src.at[:, rows(i, 16), :], raw.at[:, rows(i, 16), :], wsem.at[3 * NT + i])]
        n = src.shape[0] // 2 // parts
        if which >= 4:
            nc = raw.shape[1]
            return [pltpu.make_async_copy(
                src.at[rows(a * parts + i, n), b * nc:(b + 1) * nc], raw.at[rows((1 + q) * parts + i, n), :],
                wsem.at[4 * NT + i]) for q, (a, b) in enumerate(QUADRANTS)]
        return [pltpu.make_async_copy(
            src.at[rows(a * parts + i, n), c0:c0 + raw.shape[2]], raw.at[a, rows(i, n), :],
            wsem.at[which * NT + i]) for a in (0, 1)]

    def start(which, i):
        for c in w_copies(which, i):
            c.start()

    def wait(which, i):
        for c in w_copies(which, i):
            c.wait()

    def normalize(src, i, part=0, parts=1):
        n = M // parts
        top, bottom = (_layernorm(src[pl.ds(pl.multiple_of(i * T + r + part * n, n), n), :].astype(f32))
                       for r in (0, M))
        for t, a in enumerate(_lhs_terms(top[:, :D // 2], top[:, D // 2:], bottom[:, :D // 2], bottom[:, D // 2:])):
            n_v[i, t, rows(part, n // 2), :] = a

    def project(i, w_ref, dst, r0, order):
        first = {}
        for c0 in range(0, hb, hb // NS):
            cols = slice(128 * c0, 128 * (c0 + hb // NS))
            y = _strassen(lambda t: n_v[i, t], lambda t: w_ref[t, :, cols], order)
            for (a, b), c in zip(QUADRANTS, y):
                for j in range(hb // NS):
                    dst[b * hb + c0 + j, pl.ds(r0 + a * M, M), :] = c[:, 128 * j:128 * (j + 1)]
                    if a == 0:
                        first[b * hb + c0 + j] = c[0:1, 128 * j:128 * (j + 1)]
        return first

    def start_slabs(i):
        for which in (0, 2, 3):
            start(which, i)

    start(1, 0)
    x_copy(0).start()

    with jax.named_scope("sc_1_permk"):
        @pl.loop(0, NK)
        def _(i):
            @pl.when(i == 0)
            def _():
                x_copy(0).wait()
                start(1, 1)

            wait(1, i)

            @pl.when(i + 2 < NK)
            def _():
                start(1, i + 2)

            @pl.when(i + 2 >= NK)
            def _():
                x_copy(i + 3 - NK).start()
                start_slabs(i + 2 - NK)

            n = D // 2 // NK
            _prepare_qkv([(raw_v[1], wk_v)], pl.multiple_of(i * n, n), n)
            normalize(x_v, 0, i, NK)

    with jax.named_scope("sc_2_k"):
        @pl.loop(0, NT)
        def _(i):
            @pl.when(i + 3 < NT)
            def _():
                x_copy(i + 3).start()

            @pl.when(i + 2 < NT)
            def _():
                start_slabs(i + 2)

            for n, which in enumerate((4, 5, 6)):
                @pl.when(i == FS + n)
                def _():
                    start(which, 0)

            @pl.when(i + 1 < NT)
            def _():
                x_copy(i + 1).wait()

            for which in (0, 2, 3):
                wait(which, i)
            project(i, wk_v, k_v, pl.multiple_of(i * T, T) + HALO, OK)
            for part in range(LP):
                normalize(x_v, (i + 1) % NT, part, LP)
            pairs = [(raw_v[0], wq_v), (raw_v[2], wv_v)]
            for group in ([pairs] if JOIN else [pairs[:1], pairs[1:]]):
                _prepare_qkv(group, pl.multiple_of(i * slab, slab), slab)
            _prepare_wo(raw_v[3], wo_v, i)

    with jax.named_scope("sc_3_halo"):
        for j in range(NB):
            k_v[j, 0:HALO, :] = jnp.broadcast_to(k_v[j, HALO:HALO + 1, :], (HALO, 128))
            v_v[j, NH * T:NH * T + HALO, :] = jnp.zeros((HALO, 128), f32)

    with jax.named_scope("sc_4_attn"):
        @pl.loop(0, na)
        def _(i):
            @pl.when(i + 1 < na)
            def _():
                for which in (4, 5, 6):
                    start(which, i + 1)

            for which in (4, 5, 6):
                wait(which, i)
            r0 = pl.multiple_of(i * (NH * T), NH * T)
            v_v[:, 0:HALO, :] = v_v[:, NH * T:NH * T + HALO, :]
            salt = [0]

            def opaque(c, n):
                salt[0] += 1
                return pl.multiple_of(jnp.minimum(i + (c + salt[0]), c), n)

            def values(a):
                first = project(i * NH + a, wv_v, v_v, HALO + a * T, OV)
                if a == 0:
                    for j in range(NB):
                        v_v[j, 0:HALO, :] = jnp.where(i > 0, v_v[j, 0:HALO, :], jnp.broadcast_to(first[j], (HALO, 128)))

            def attend(a):
                for c in range(0, M, R):
                    o1, o2 = (_attend(q_v, k_v, v_v, r, r0 + (opaque(r, R) if OPQ[0] else r),
                                      opaque(r, R) if OPQ[1] else r, r0 + r if r < HALO else None)
                              for r in (a * T + c, a * T + M + c))
                    for j in range(hb):
                        for t, y in enumerate(_lhs_terms(o1[j], o1[j + hb], o2[j], o2[j + hb])):
                            o_v[a, t, c // 2:(c + R) // 2, 128 * j:128 * (j + 1)] = y

            def out_proj(a):
                y = _strassen(lambda t: o_v[a, t], lambda t: wo_v[t], OO)
                for (ra, b), c in zip(QUADRANTS, y):
                    rr, cc = pl.ds(r0 + a * T + ra * M, M), slice(b * (D // 2), (b + 1) * (D // 2))
                    h_v[rr, cc] = x_v[rr, cc].astype(f32) + c

            steps = dict(q=lambda a: project(i * NH + a, wq_v, q_v, a * T, OQ), v=values, a=attend, o=out_proj)
            for step in ORDER.split():
                steps[step[0]](int(step[1]))
            if PC:
                for which in (4, 5, 6):
                    w_ref = raw_v[which]
                    n = w_ref.shape[0] // 7 // na
                    for c in range(0, n, 16):
                        for c0 in range(0, w_ref.shape[1], PC):
                            _prepare_ffn(w_ref, pl.multiple_of(i * n, 16) + opaque(c, 16), c0,
                                         min(PC, w_ref.shape[1] - c0))

    with jax.named_scope("sc_5_ln"):
        @pl.loop(0, 2)
        def _(part):
            normalize(h_v, 0, part, 2)

    with jax.named_scope("sc_6_ffn"):
        @pl.loop(0, NT)
        def _(i):
            for n, c in enumerate(range(0, F // 2 if FFN else FC, FC)):
                g = _strassen(lambda t: n_v[i, t], lambda t: _words(raw_v[4][t * (D // 2):(t + 1) * (D // 2), c:c + FC]), OG)
                u = _strassen(lambda t: n_v[i, t], lambda t: _words(raw_v[5][t * (D // 2):(t + 1) * (D // 2), c:c + FC]), OG)
                act = [jax.nn.gelu(a, approximate=True) * b for a, b in zip(g, u)]
                for t, a in enumerate(_lhs_terms(*act)):
                    act_v[t, :, c:c + FC] = a
            normalize(h_v, (i + 1) % NT)
            y = _strassen(lambda t: act_v[t], lambda t: _words(raw_v[6][t * (F // 2):(t + 1) * (F // 2), :]), OD)
            for (a, b), c in zip(QUADRANTS, y):
                rr, cc = pl.ds(pl.multiple_of(i * T, T) + a * M, M), slice(b * (D // 2), (b + 1) * (D // 2))
                out_v[rr, cc] = (h_v[rr, cc] + c).astype(bf16)
            out_copy(i).start()

    with jax.named_scope("sc_7_out"):
        for i in range(NT):
            out_copy(i).wait()


@jax.jit
def pallas_sequential_preLN__sliding_local_dilated__glu_gated_geglu__prompt_kernel(
        A_x, A_wqkv, A_wo, B_x, B_w_gate, B_w_up, B_w_down):
    del B_x
    any_spec = pl.BlockSpec(memory_space=pl.ANY)
    terms = lambda k, n: pltpu.VMEM((7, k // 4, n // 2), i32)
    na = NT // NH
    out = pl.pallas_call(
        _kernel,
        in_specs=[any_spec] * 6,
        out_specs=any_spec,
        out_shape=jax.ShapeDtypeStruct((S, D), bf16),
        scratch_shapes=[
            pltpu.VMEM((S, D), bf16),
            [pltpu.VMEM((2, D // 2, D), bf16)] * 3 + [pltpu.VMEM((NB, 128, D), bf16)]
            + [pltpu.VMEM((7 * D // 2, F // 2), bf16)] * 2
            + [pltpu.VMEM((7 * F // 2, D // 2), bf16)],
            pltpu.VMEM((NT, 7, M // 2, D // 2), i32),
            terms(D, D), terms(D, D), terms(D, D), terms(D, D),
            pltpu.VMEM((NB, NH * T, 128), f32), pltpu.VMEM((NB, S + HALO, 128), f32),
            pltpu.VMEM((NB, NH * T + HALO, 128), f32), pltpu.VMEM((NH, 7, M // 2, D // 2), i32),
            pltpu.VMEM((S, D), f32), terms(T, F),
            pltpu.SemaphoreType.DMA((NT,)), pltpu.SemaphoreType.DMA((4 * NT + na,)),
            pltpu.SemaphoreType.DMA,
        ],
        compiler_params=pltpu.CompilerParams(vmem_limit_bytes=120 * 1024 * 1024, flags=FLAGS, disable_bounds_checks=NOCHK),
    )(A_x.reshape(S, D), A_wqkv, A_wo.reshape(NB, 128, D), B_w_gate, B_w_up, B_w_down)
    return out.reshape(1, S, D)
```

```python
import jax
import jax.numpy as jnp
import jax.experimental.pallas as pl
import jax.experimental.pallas.tpu as pltpu

S, D, F = 2048, 1024, 3584
HEAD_DIM, WINDOW, DILATION = 32, 8, 2
EPS = 1e-5
NB = D // 128
HALO = 16
T = 256
M = T // 2
NT = S // T
NH = 2
R = 32
FC = 256
OK = OV = OQ = OO = OG = OD = '1304265'
NS = 1
CHAIN = 'qnv'
LP1 = 2
LP2 = 8
FS = 3
FLAGS = None
ORDER = 'v0 q0 v1 q1 a0 a1 o0 o1'
TREE = 0
OPQ = (0, 0)
FFN = 1
PC = 512
NOCHK = True
NK = 4
f32, bf16, i32 = jnp.float32, jnp.bfloat16, jnp.int32

QUADRANTS = ((0, 0), (0, 1), (1, 0), (1, 1))


def _words(x):
    return pltpu.bitcast(x.astype(bf16), i32)


def _dot(a, b):
    return jnp.dot(pltpu.bitcast(a, bf16), pltpu.bitcast(b, bf16), preferred_element_type=f32)


def _layernorm(x):
    c = x - jnp.mean(x, axis=-1, keepdims=True)
    return c * jax.lax.rsqrt(jnp.mean(c * c, axis=-1, keepdims=True) + EPS)


def _lane_xor(x, bits):
    lane = jax.lax.broadcasted_iota(jnp.int32, x.shape, 1)
    return jnp.take_along_axis(x, lane ^ bits, axis=1, mode="promise_in_bounds")


def _exchange_lanes(blocks):
    lane = jax.lax.broadcasted_iota(jnp.int32, blocks[0].shape, 1)
    blocks = [_lane_xor(b, 2 * j) if j else b for j, b in enumerate(blocks)]
    for t in (1, 2, 4):
        hi = (lane & (2 * t)) != 0
        blocks = [jnp.where(hi, blocks[j ^ t], blocks[j]) for j in range(NB)]
    return [_lane_xor(b, 2 * j) if j else b for j, b in enumerate(blocks)]


def _exchange_rows(blocks):
    row = jax.lax.broadcasted_iota(jnp.int32, blocks[0].shape, 0)
    for t in (1, 2, 4):
        hi = (row & t) != 0
        blocks = [jnp.where(hi, blocks[j], pltpu.roll(blocks[j ^ t], 8 - t, 0)) if j & t else
                  jnp.where(hi, pltpu.roll(blocks[j ^ t], t, 0), blocks[j]) for j in range(NB)]
    return blocks


def _rhs_terms(b11, b12, b21, b22):
    c11, c12, c21, c22 = (b.astype(f32) for b in (b11, b12, b21, b22))
    return [_words(t) for t in (c11 + c22, b11, c12 - c22, c21 - c11, b22, c11 + c12, c21 + c22)]


def _lhs_terms(a11, a12, a21, a22):
    return [_words(t) for t in (a11 + a22, a21 + a22, a11, a22, a11 + a12, a21 - a11, a12 - a22)]


BLOCKS = (((0, 1), (3, 1), (4, -1), (6, 1)), ((2, 1), (4, 1)), ((1, 1), (3, 1)), ((0, 1), (1, -1), (2, 1), (5, 1)))


def _strassen(lhs, rhs, order):
    out = [None] * 4
    for i in map(int, order):
        m = _dot(lhs(i), rhs(i))
        for q, block in enumerate(BLOCKS):
            sign = dict(block).get(i)
            if sign is None:
                continue
            if out[q] is None:
                out[q] = (m, sign)
            else:
                acc, s = out[q]
                out[q] = (acc + m, s) if s == sign else (acc - m, 1) if s > 0 else (m - acc, 1)
    return [acc for acc, _ in out]


def _prepare_qkv(pairs, r, n):
    hb, k = NB // 2, n // 2
    blocks = _exchange_lanes([
        jnp.concatenate([_words(raw[a, pl.ds(r, n), 128 * j:128 * (j + 1)]) for raw, _ in pairs for a in (0, 1)])
        for j in range(NB)])
    for p, (_, w_ref) in enumerate(pairs):
        for j in range(hb):
            quads = [pltpu.bitcast(blocks[j + b * hb][(2 * p + a) * k:(2 * p + a + 1) * k], bf16)
                     for a, b in QUADRANTS]
            for i, t in enumerate(_rhs_terms(*quads)):
                w_ref[i, pl.ds(pl.multiple_of(r // 2, 8), k), 128 * j:128 * (j + 1)] = t
    return t


def _prepare_wo(raw, w_ref, m):
    hb = NB // 2
    for c in range(0, D // 2, 128):
        halves = []
        for c0 in (c, D // 2 + c):
            blocks = [_words(raw[j, pl.ds(pl.multiple_of(16 * m, 16), 16), c0:c0 + 128]) for j in range(NB)]
            halves.append([pltpu.bitcast(t, bf16) for t in _exchange_rows(blocks)])
        for j in range(hb):
            for i, t in enumerate(_rhs_terms(halves[0][j], halves[1][j], halves[0][j + hb], halves[1][j + hb])):
                w_ref[i, pl.ds(pl.multiple_of(64 * j + 8 * m, 8), 8), c:c + 128] = t


def _prepare_ffn(w_ref, r, c, n):
    nr = w_ref.shape[0] // 7
    at = lambda i: (pl.ds(i * nr + r, 16), slice(c, c + n))
    terms = _rhs_terms(*(w_ref[at(i)] for i in (1, 2, 3, 4)))
    for i in (0, 2, 3, 5, 6):
        w_ref[at(i)] = pltpu.bitcast(terms[i], bf16)


def _sum(t):
    if not TREE:
        acc = t[0]
        for a in t[1:]:
            acc = acc + a
        return acc
    while len(t) > 1:
        t = [a + b for a, b in zip(t[::2], t[1::2])]
    return t[0]


def _softmax(sums, pos):
    logits = []
    for w, s in enumerate(sums):
        for b in (1, 16):
            s = s + _lane_xor(s, b)
        s = s * HEAD_DIM ** -0.5
        if pos is not None and w:
            s = jnp.where(pos + jax.lax.broadcasted_iota(i32, s.shape, 0) >= DILATION * w, s, -1e9)
        logits.append(s)
    top = logits[0]
    for s in logits[1:]:
        top = jnp.maximum(top, s)
    e = [jnp.exp(s - top) for s in logits]
    den = e[0]
    for t in e[1:]:
        den = den + t
    inv = 1.0 / den
    return [t * inv for t in e]


def _attend(q_ref, k_ref, v_ref, r, kr, vr, pos):
    window = lambda ref, j, r0, w: ref[j, pl.ds(r0 + HALO - DILATION * w, R), :]
    q = [q_ref[j, r:r + R, :] for j in range(NB)]
    p = _softmax([_sum([q[j] * window(k_ref, j, kr, w) for j in range(NB)]) for w in range(WINDOW)], pos)
    return [_sum([p[w] * window(v_ref, j, vr, w) for w in range(WINDOW)]) for j in range(NB)]


def _kernel(x_hbm, wqkv_hbm, wo_hbm, wg_hbm, wu_hbm, wd_hbm, out_hbm,
            x_v, raw_v, n_v, wq_v, wk_v, wv_v, wo_v, q_v, k_v, v_v, o_v, h_v, act_v,
            xsem, wsem, osem):
    hb = NB // 2
    na = NT // NH
    out_v = x_v
    slab = D // 2 // NT

    def rows(i, n):
        return pl.ds(pl.multiple_of(i * n, n), n)

    def x_copy(i):
        return pltpu.make_async_copy(x_hbm.at[rows(i, T), :], x_v.at[rows(i, T), :], xsem.at[i])

    def out_copy(i):
        return pltpu.make_async_copy(out_v.at[rows(i, T), :], out_hbm.at[rows(i, T), :], osem)

    weights = ((wqkv_hbm, 0, NT), (wqkv_hbm, D, NK), (wqkv_hbm, 2 * D, NT),
               (wo_hbm, 0, NT), (wg_hbm, 0, na), (wu_hbm, 0, na), (wd_hbm, 0, na))

    def w_copies(which, i):
        src, c0, parts = weights[which]
        raw = raw_v[which]
        if which == 3:
            return [pltpu.make_async_copy(src.at[:, rows(i, 16), :], raw.at[:, rows(i, 16), :], wsem.at[3 * NT + i])]
        n = src.shape[0] // 2 // parts
        if which >= 4:
            nc = raw.shape[1]
            return [pltpu.make_async_copy(
                src.at[rows(a * parts + i, n), b * nc:(b + 1) * nc], raw.at[rows((1 + q) * parts + i, n), :],
                wsem.at[4 * NT + i]) for q, (a, b) in enumerate(QUADRANTS)]
        return [pltpu.make_async_copy(
            src.at[rows(a * parts + i, n), c0:c0 + raw.shape[2]], raw.at[a, rows(i, n), :],
            wsem.at[which * NT + i]) for a in (0, 1)]

    def start(which, i):
        for c in w_copies(which, i):
            c.start()

    def wait(which, i):
        for c in w_copies(which, i):
            c.wait()

    def normalize(src, i, part=0, parts=1):
        n = M // parts
        top, bottom = (_layernorm(src[pl.ds(pl.multiple_of(i * T + r + part * n, n), n), :].astype(f32))
                       for r in (0, M))
        for t, a in enumerate(_lhs_terms(top[:, :D // 2], top[:, D // 2:], bottom[:, :D // 2], bottom[:, D // 2:])):
            n_v[i, t, rows(part, n // 2), :] = a
        return a

    def normalize_staggered(src, i, parts):
        for part in range(parts):
            token = normalize(src, i, part, parts)
            spare = pl.multiple_of(jnp.minimum(S + part + i, S), 16)
            if src.dtype == bf16:
                src[pl.ds(spare, 16), 0:128] = pltpu.bitcast(token[-8:, -128:], bf16)
            else:
                src[pl.ds(spare, 8), 0:128] = pltpu.bitcast(token[-8:, -128:], f32)
        return token

    def project(i, w_ref, dst, r0, order):
        first = {}
        for c0 in range(0, hb, hb // NS):
            cols = slice(128 * c0, 128 * (c0 + hb // NS))
            y = _strassen(lambda t: n_v[i, t], lambda t: w_ref[t, :, cols], order)
            for (a, b), c in zip(QUADRANTS, y):
                for j in range(hb // NS):
                    dst[b * hb + c0 + j, pl.ds(r0 + a * M, M), :] = c[:, 128 * j:128 * (j + 1)]
                    if a == 0:
                        first[b * hb + c0 + j] = c[0:1, 128 * j:128 * (j + 1)]
        return first

    def start_slabs(i):
        for which in (0, 2, 3):
            start(which, i)

    start(1, 0)
    x_copy(0).start()

    with jax.named_scope("sc_1_permk"):
        @pl.loop(0, NK)
        def _(i):
            @pl.when(i == 0)
            def _():
                x_copy(0).wait()
                start(1, 1)

            wait(1, i)

            @pl.when(i + 2 < NK)
            def _():
                start(1, i + 2)

            @pl.when(i + 2 >= NK)
            def _():
                x_copy(i + 3 - NK).start()
                start_slabs(i + 2 - NK)

            n = D // 2 // NK
            _prepare_qkv([(raw_v[1], wk_v)], pl.multiple_of(i * n, n), n)
            normalize(x_v, 0, i, NK)

    with jax.named_scope("sc_2_k"):
        @pl.loop(0, NT)
        def _(i):
            @pl.when(i + 3 < NT)
            def _():
                x_copy(i + 3).start()

            @pl.when(i + 2 < NT)
            def _():
                start_slabs(i + 2)

            for n, which in enumerate((4, 5, 6)):
                @pl.when(i == FS + n)
                def _():
                    start(which, 0)

            @pl.when(i + 1 < NT)
            def _():
                x_copy(i + 1).wait()

            for which in (0, 2, 3):
                wait(which, i)
            project(i, wk_v, k_v, pl.multiple_of(i * T, T) + HALO, OK)
            token = None
            for step in CHAIN:
                if step == '-':
                    token = None
                    continue
                if step == 'n':
                    token = normalize_staggered(x_v, (i + 1) % NT, LP1)
                    continue
                raw, w_ref = dict(q=(raw_v[0], wq_v), v=(raw_v[2], wv_v))[step]
                if token is not None:
                    for a in (0, 1):
                        spare = pl.multiple_of(jnp.minimum(D // 2 + i, D // 2), 16)
                        raw[a, pl.ds(spare, 16), 0:128] = pltpu.bitcast(token[-8:, -128:], bf16)
                token = _prepare_qkv([(raw, w_ref)], pl.multiple_of(i * slab, slab), slab)
            _prepare_wo(raw_v[3], wo_v, i)

    with jax.named_scope("sc_3_halo"):
        for j in range(NB):
            k_v[j, 0:HALO, :] = jnp.broadcast_to(k_v[j, HALO:HALO + 1, :], (HALO, 128))
            v_v[j, NH * T:NH * T + HALO, :] = jnp.zeros((HALO, 128), f32)

    with jax.named_scope("sc_4_attn"):
        @pl.loop(0, na)
        def _(i):
            @pl.when(i + 1 < na)
            def _():
                for which in (4, 5, 6):
                    start(which, i + 1)

            for which in (4, 5, 6):
                wait(which, i)
            r0 = pl.multiple_of(i * (NH * T), NH * T)
            v_v[:, 0:HALO, :] = v_v[:, NH * T:NH * T + HALO, :]
            salt = [0]

            def opaque(c, n):
                salt[0] += 1
                return pl.multiple_of(jnp.minimum(i + (c + salt[0]), c), n)

            def values(a):
                first = project(i * NH + a, wv_v, v_v, HALO + a * T, OV)
                if a == 0:
                    for j in range(NB):
                        v_v[j, 0:HALO, :] = jnp.where(i > 0, v_v[j, 0:HALO, :], jnp.broadcast_to(first[j], (HALO, 128)))

            def attend(a):
                for c in range(0, M, R):
                    o1, o2 = (_attend(q_v, k_v, v_v, r, r0 + (opaque(r, R) if OPQ[0] else r),
                                      opaque(r, R) if OPQ[1] else r, r0 + r if r < HALO else None)
                              for r in (a * T + c, a * T + M + c))
                    for j in range(hb):
                        for t, y in enumerate(_lhs_terms(o1[j], o1[j + hb], o2[j], o2[j + hb])):
                            o_v[a, t, c // 2:(c + R) // 2, 128 * j:128 * (j + 1)] = y

            def out_proj(a):
                y = _strassen(lambda t: o_v[a, t], lambda t: wo_v[t], OO)
                for (ra, b), c in zip(QUADRANTS, y):
                    rr, cc = pl.ds(r0 + a * T + ra * M, M), slice(b * (D // 2), (b + 1) * (D // 2))
                    h_v[rr, cc] = x_v[rr, cc].astype(f32) + c

            steps = dict(q=lambda a: project(i * NH + a, wq_v, q_v, a * T, OQ), v=values, a=attend, o=out_proj)
            for step in ORDER.split():
                steps[step[0]](int(step[1]))
            if PC:
                for which in (4, 5, 6):
                    w_ref = raw_v[which]
                    n = w_ref.shape[0] // 7 // na
                    for c in range(0, n, 16):
                        for c0 in range(0, w_ref.shape[1], PC):
                            _prepare_ffn(w_ref, pl.multiple_of(i * n, 16) + opaque(c, 16), c0,
                                         min(PC, w_ref.shape[1] - c0))

    with jax.named_scope("sc_5_ln"):
        @pl.loop(0, 2)
        def _(part):
            normalize(h_v, 0, part, 2)

    with jax.named_scope("sc_6_ffn"):
        @pl.loop(0, NT)
        def _(i):
            for n, c in enumerate(range(0, F // 2 if FFN else FC, FC)):
                g = _strassen(lambda t: n_v[i, t], lambda t: _words(raw_v[4][t * (D // 2):(t + 1) * (D // 2), c:c + FC]), OG)
                u = _strassen(lambda t: n_v[i, t], lambda t: _words(raw_v[5][t * (D // 2):(t + 1) * (D // 2), c:c + FC]), OG)
                act = [jax.nn.gelu(a, approximate=True) * b for a, b in zip(g, u)]
                for t, a in enumerate(_lhs_terms(*act)):
                    act_v[t, :, c:c + FC] = a
            normalize_staggered(h_v, (i + 1) % NT, LP2)
            y = _strassen(lambda t: act_v[t], lambda t: _words(raw_v[6][t * (F // 2):(t + 1) * (F // 2), :]), OD)
            for (a, b), c in zip(QUADRANTS, y):
                rr, cc = pl.ds(pl.multiple_of(i * T, T) + a * M, M), slice(b * (D // 2), (b + 1) * (D // 2))
                out_v[rr, cc] = (h_v[rr, cc] + c).astype(bf16)
            out_copy(i).start()

    with jax.named_scope("sc_7_out"):
        for i in range(NT):
            out_copy(i).wait()


@jax.jit
def pallas_sequential_preLN__sliding_local_dilated__glu_gated_geglu__prompt_kernel(
        A_x, A_wqkv, A_wo, B_x, B_w_gate, B_w_up, B_w_down):
    del B_x
    any_spec = pl.BlockSpec(memory_space=pl.ANY)
    terms = lambda k, n: pltpu.VMEM((7, k // 4, n // 2), i32)
    na = NT // NH
    out = pl.pallas_call(
        _kernel,
        in_specs=[any_spec] * 6,
        out_specs=any_spec,
        out_shape=jax.ShapeDtypeStruct((S, D), bf16),
        scratch_shapes=[
            pltpu.VMEM((S + 16, D), bf16),
            [pltpu.VMEM((2, D // 2 + 16, D), bf16)] * 3 + [pltpu.VMEM((NB, 128, D), bf16)]
            + [pltpu.VMEM((7 * D // 2, F // 2), bf16)] * 2
            + [pltpu.VMEM((7 * F // 2, D // 2), bf16)],
            pltpu.VMEM((NT, 7, M // 2, D // 2), i32),
            terms(D, D), terms(D, D), terms(D, D), terms(D, D),
            pltpu.VMEM((NB, NH * T, 128), f32), pltpu.VMEM((NB, S + HALO, 128), f32),
            pltpu.VMEM((NB, NH * T + HALO, 128), f32), pltpu.VMEM((NH, 7, M // 2, D // 2), i32),
            pltpu.VMEM((S + 8, D), f32), terms(T, F),
            pltpu.SemaphoreType.DMA((NT,)), pltpu.SemaphoreType.DMA((4 * NT + na,)),
            pltpu.SemaphoreType.DMA,
        ],
        compiler_params=pltpu.CompilerParams(vmem_limit_bytes=120 * 1024 * 1024, flags=FLAGS, disable_bounds_checks=NOCHK),
    )(A_x.reshape(S, D), A_wqkv, A_wo.reshape(NB, 128, D), B_w_gate, B_w_up, B_w_down)
    return out.reshape(1, S, D)
```

```python
import jax
import jax.numpy as jnp
import jax.experimental.pallas as pl
import jax.experimental.pallas.tpu as pltpu

S, D, F = 2048, 1024, 3584
HEAD_DIM, WINDOW, DILATION = 32, 8, 2
EPS = 1e-5
SCALE = HEAD_DIM ** -0.5
LOG2E = 1.4426950408889634
NB = D // 128
HALO = 16
T = 256
M = T // 2
NT = S // T
NH = 2
R = 32
FC = 256
OK = OG = '1304265'
OV, OQ, OO = '1302546', '1302564', '2403651'
OD = '1302546'
NS = 2
CHAIN = 'q-nv'
LP1 = 2
LP2 = 8
EARLY = 1
ROLL = 0
QS = 1
LATE = 1
NQ, NV, NO = 4, 2, 2
OQ1 = OO1 = '1304265'
FLAGS = None
ORDER = 'v0 q0 q1 v1 a0 a1 o0 o1'
TREE = 1
OPQ = (0, 0)
FFN = 1
PC = 512
NOCHK = False
NK = 4
f32, bf16, i32 = jnp.float32, jnp.bfloat16, jnp.int32

QUADRANTS = ((0, 0), (0, 1), (1, 0), (1, 1))


def _words(x):
    return pltpu.bitcast(x.astype(bf16), i32)


def _dot(a, b):
    return jnp.dot(pltpu.bitcast(a, bf16), pltpu.bitcast(b, bf16), preferred_element_type=f32)


def _layernorm(x):
    c = x - jnp.mean(x, axis=-1, keepdims=True)
    return c * jax.lax.rsqrt(jnp.mean(c * c, axis=-1, keepdims=True) + EPS)


def _lane_xor(x, bits):
    lane = jax.lax.broadcasted_iota(jnp.int32, x.shape, 1)
    return jnp.take_along_axis(x, lane ^ bits, axis=1, mode="promise_in_bounds")


def _exchange_lanes(blocks):
    lane = jax.lax.broadcasted_iota(jnp.int32, blocks[0].shape, 1)
    blocks = [_lane_xor(b, 2 * j) if j else b for j, b in enumerate(blocks)]
    for t in (1, 2, 4):
        hi = (lane & (2 * t)) != 0
        blocks = [jnp.where(hi, blocks[j ^ t], blocks[j]) for j in range(NB)]
    return [_lane_xor(b, 2 * j) if j else b for j, b in enumerate(blocks)]


def _exchange_lanes_roll(blocks):
    lane = jax.lax.broadcasted_iota(jnp.int32, blocks[0].shape, 1)
    for t in (1, 2, 4):
        hi = (lane & (2 * t)) != 0
        blocks = [jnp.where(hi, blocks[j], pltpu.roll(blocks[j ^ t], 128 - 2 * t, 1)) if j & t else
                  jnp.where(hi, pltpu.roll(blocks[j ^ t], 2 * t, 1), blocks[j]) for j in range(NB)]
    return blocks


def _exchange_rows(blocks):
    row = jax.lax.broadcasted_iota(jnp.int32, blocks[0].shape, 0)
    for t in (1, 2, 4):
        hi = (row & t) != 0
        blocks = [jnp.where(hi, blocks[j], pltpu.roll(blocks[j ^ t], 8 - t, 0)) if j & t else
                  jnp.where(hi, pltpu.roll(blocks[j ^ t], t, 0), blocks[j]) for j in range(NB)]
    return blocks


def _rhs_terms(b11, b12, b21, b22):
    c11, c12, c21, c22 = (b.astype(f32) for b in (b11, b12, b21, b22))
    return [_words(t) for t in (c11 + c22, b11, c12 - c22, c21 - c11, b22, c11 + c12, c21 + c22)]


def _lhs_terms(a11, a12, a21, a22):
    return [_words(t) for t in (a11 + a22, a21 + a22, a11, a22, a11 + a12, a21 - a11, a12 - a22)]


BLOCKS = (((0, 1), (3, 1), (4, -1), (6, 1)), ((2, 1), (4, 1)), ((1, 1), (3, 1)), ((0, 1), (1, -1), (2, 1), (5, 1)))


def _strassen(lhs, rhs, order):
    out = [None] * 4
    for i in map(int, order):
        m = _dot(lhs(i), rhs(i))
        for q, block in enumerate(BLOCKS):
            sign = dict(block).get(i)
            if sign is None:
                continue
            if out[q] is None:
                out[q] = (m, sign)
            else:
                acc, s = out[q]
                out[q] = (acc + m, s) if s == sign else (acc - m, 1) if s > 0 else (m - acc, 1)
    return [acc for acc, _ in out]


def _prepare_qkv(pairs, r, n, roll=False):
    hb, k = NB // 2, n // 2
    blocks = (_exchange_lanes_roll if roll else _exchange_lanes)([
        jnp.concatenate([_words(raw[a, pl.ds(r, n), 128 * j:128 * (j + 1)]) for raw, _ in pairs for a in (0, 1)])
        for j in range(NB)])
    for p, (_, w_ref) in enumerate(pairs):
        for j in range(hb):
            quads = [pltpu.bitcast(blocks[j + b * hb][(2 * p + a) * k:(2 * p + a + 1) * k], bf16)
                     for a, b in QUADRANTS]
            for i, t in enumerate(_rhs_terms(*quads)):
                w_ref[i, pl.ds(pl.multiple_of(r // 2, 8), k), 128 * j:128 * (j + 1)] = t
    return t


def _prepare_wo(raw, w_ref, m):
    hb = NB // 2
    for c in range(0, D // 2, 128):
        halves = []
        for c0 in (c, D // 2 + c):
            blocks = [_words(raw[j, pl.ds(pl.multiple_of(16 * m, 16), 16), c0:c0 + 128]) for j in range(NB)]
            halves.append([pltpu.bitcast(t, bf16) for t in _exchange_rows(blocks)])
        for j in range(hb):
            for i, t in enumerate(_rhs_terms(halves[0][j], halves[1][j], halves[0][j + hb], halves[1][j + hb])):
                w_ref[i, pl.ds(pl.multiple_of(64 * j + 8 * m, 8), 8), c:c + 128] = t


def _prepare_ffn(w_ref, r, c, n):
    nr = w_ref.shape[0] // 7
    at = lambda i: (pl.ds(i * nr + r, 16), slice(c, c + n))
    terms = _rhs_terms(*(w_ref[at(i)] for i in (1, 2, 3, 4)))
    for i in (0, 2, 3, 5, 6):
        w_ref[at(i)] = pltpu.bitcast(terms[i], bf16)


def _sum(t):
    if not TREE:
        acc = t[0]
        for a in t[1:]:
            acc = acc + a
        return acc
    while len(t) > 1:
        t = [a + b for a, b in zip(t[::2], t[1::2])]
    return t[0]


def _softmax(sums, pos):
    logits = []
    for w, s in enumerate(sums):
        for b in (1, 16):
            s = s + _lane_xor(s, b)
        if pos is not None and w:
            s = jnp.where(pos + jax.lax.broadcasted_iota(i32, s.shape, 0) >= DILATION * w, s, -1e9 / SCALE)
        logits.append(s)
    top = logits[0]
    for s in logits[1:]:
        top = jnp.maximum(top, s)
    e = [jnp.exp2((s - top) * (SCALE * LOG2E)) for s in logits]
    den = _sum(e)
    inv = pl.reciprocal(den, approx=True)
    inv = inv * (2.0 - den * inv)
    return [t * inv for t in e]


def _attend(q_ref, k_ref, v_ref, r, kr, vr, pos):
    window = lambda ref, j, r0, w: ref[j, pl.ds(r0 + HALO - DILATION * w, R), :]
    q = [q_ref[j, r:r + R, :] for j in range(NB)]
    p = _softmax([_sum([q[j] * window(k_ref, j, kr, w) for j in range(NB)]) for w in range(WINDOW)], pos)
    return [_sum([p[w] * window(v_ref, j, vr, w) for w in range(WINDOW)]) for j in range(NB)]


def _kernel(x_hbm, wqkv_hbm, wo_hbm, wg_hbm, wu_hbm, wd_hbm, out_hbm,
            x_v, raw_v, n_v, wq_v, wk_v, wv_v, wo_v, q_v, k_v, v_v, o_v, h_v, act_v,
            fsem, ksem, xsem, wsem, osem):
    hb = NB // 2
    na = NT // NH
    out_v = x_v
    slab = D // 2 // NT

    def rows(i, n):
        if isinstance(i, int):
            return pl.ds(i * n, n)
        return pl.ds(pl.multiple_of(i * n, n), n)

    copy = pltpu.make_async_copy

    def halves(col, parts, i, sem):
        r = rows(i, D // 2 // parts)
        return copy(wqkv_hbm.at[:, r, col * D:(col + 1) * D], raw_v[col].at[:, r, :], sem)

    def x_rows(i, n, sem):
        return copy(x_hbm.at[rows(i, n), :], x_v.at[rows(i, n), :], sem)

    def first_copies(i, step):
        sem = fsem.at[step % 2]
        return [halves(1, NK, i, sem), x_rows(i, M // NK, sem), x_rows(NK + i, M // NK, sem)]

    def key_copies(i, step):
        sem = ksem.at[step % 4]
        return [halves(0, NT, i, sem), halves(2, NT, i, sem),
                copy(wo_hbm.at[:, rows(i, 16), :], raw_v[3].at[:, rows(i, 16), :], sem)]

    def x_copies(i, step):
        return [x_rows(i, T, xsem.at[step % 4])]

    def ffn_copies(i, step, halves=(0, 1)):
        out = []
        for src, dst in ((wg_hbm, raw_v[4]), (wu_hbm, raw_v[5]), (wd_hbm, raw_v[6])):
            n, nc = dst.shape[0] // 7 // na, dst.shape[1]
            for a in halves:
                for b in (0, 1):
                    out.append(copy(src.at[rows(a * na + i, n), b * nc:(b + 1) * nc],
                                    dst.at[rows((1 + 2 * a + b) * na + i, n), :], wsem.at[step % 2]))
        return out

    def out_copy(r):
        return copy(out_v.at[pl.ds(r, M), :], out_hbm.at[pl.ds(r, M), :], osem)

    def start(copies, i, *args):
        for c in copies(i, i, *args):
            c.start()

    def wait(copies, i):
        for c in copies(0, i):
            c.wait()

    def normalize(src, i, part=0, parts=1):
        n = M // parts
        top, bottom = (_layernorm(src[pl.ds(pl.multiple_of(i % NT * T + r + part * n, n), n), :].astype(f32))
                       for r in (0, M))
        for t, a in enumerate(_lhs_terms(top[:, :D // 2], top[:, D // 2:], bottom[:, :D // 2], bottom[:, D // 2:])):
            n_v[i, t, rows(part, n // 2), :] = a
        return a

    def hand_over(ref, i, step, token):
        spare = pl.multiple_of(jnp.minimum(S + step + i, S), 16)
        if ref.dtype == bf16:
            ref[pl.ds(spare, 16), 0:128] = pltpu.bitcast(token[-8:, -128:], bf16)
        else:
            ref[pl.ds(spare, 8), 0:128] = pltpu.bitcast(token[-8:, -128:], f32)

    def normalize_staggered(src, i, parts):
        for part in range(parts):
            token = normalize(src, i, part, parts)
            hand_over(src, i, part, token)
        return token

    def project(i, w_ref, dst, r0, order, NS, lhs=None):
        row0 = {}
        for c0 in range(0, hb, hb // NS):
            cols = slice(128 * c0, 128 * (c0 + hb // NS))
            y = _strassen(lhs or (lambda t: n_v[i, t]), lambda t: w_ref[t, :, cols], order)
            for (a, b), c in zip(QUADRANTS, y):
                for j in range(hb // NS):
                    dst[b * hb + c0 + j, pl.ds(r0 + a * M, M), :] = c[:, 128 * j:128 * (j + 1)]
                    if a == 0:
                        row0[b * hb + c0 + j] = c[0:1, 128 * j:128 * (j + 1)]
        return row0

    start(first_copies, 0)
    start(first_copies, 1)

    with jax.named_scope("sc_1_permk"):
        @pl.loop(0, NK)
        def _(i):
            wait(first_copies, i)

            @pl.when(i + 2 < NK)
            def _():
                start(first_copies, i + 2)

            @pl.when(i + 2 >= NK)
            def _():
                start(key_copies, i + 2 - NK)
                start(x_copies, i + 3 - NK)

            n = D // 2 // NK
            _prepare_qkv([(raw_v[1], wk_v)], pl.multiple_of(i * n, n), n)
            normalize(x_v, 0, i, NK)

    with jax.named_scope("sc_2_k"):
        @pl.loop(0, NT)
        def _(i):
            @pl.when(i + 3 < NT)
            def _():
                start(x_copies, i + 3)

            @pl.when(i + 2 < NT)
            def _():
                start(key_copies, i + 2)

            for a in (0, 1):
                @pl.when(i == NT - 3 + a)
                def _():
                    start(ffn_copies, 0, [a])

            @pl.when(i + 1 < NT)
            def _():
                wait(x_copies, i + 1)

            wait(key_copies, i)
            project(i, wk_v, k_v, pl.multiple_of(i * T, T) + HALO, OK, NS)
            token = None
            for step in CHAIN:
                if step == '-':
                    token = None
                    continue
                if step == 'n':
                    token = normalize_staggered(x_v, i + 1, LP1)
                    continue
                raw, w_ref = dict(q=(raw_v[0], wq_v), v=(raw_v[2], wv_v))[step]
                for part in range(QS):
                    if token is not None:
                        for a in (0, 1):
                            spare = pl.multiple_of(jnp.minimum(D // 2 + i + part, D // 2), 16)
                            raw[a, pl.ds(spare, 16), 0:128] = pltpu.bitcast(token[-8:, -128:], bf16)
                    n = slab // QS
                    token = _prepare_qkv([(raw, w_ref)], pl.multiple_of(i * slab + part * n, n), n, ROLL)
            _prepare_wo(raw_v[3], wo_v, i)

    with jax.named_scope("sc_3_halo"):
        for j in range(NB):
            k_v[j, 0:HALO, :] = jnp.broadcast_to(k_v[j, HALO:HALO + 1, :], (HALO, 128))
            v_v[j, NH * T:NH * T + HALO, :] = jnp.zeros((HALO, 128), f32)

    with jax.named_scope("sc_4_attn"):
        @pl.loop(0, na)
        def _(i):
            if LATE:
                for n in range(1, na):
                    @pl.when(i + 1 == n)
                    def _():
                        start(ffn_copies, n)
            else:
                @pl.when(i + 1 < na)
                def _():
                    start(ffn_copies, i + 1)

            wait(ffn_copies, i)
            r0 = pl.multiple_of(i * (NH * T), NH * T)
            v_v[:, 0:HALO, :] = v_v[:, NH * T:NH * T + HALO, :]
            salt = [0]

            def opaque(c, n):
                salt[0] += 1
                return pl.multiple_of(jnp.minimum(i + (c + salt[0]), c), n)

            def values(a):
                row0 = project(i * NH + a, wv_v, v_v, HALO + a * T, OV, NV)
                if a == 0:
                    for j in range(NB):
                        v_v[j, 0:HALO, :] = jnp.where(i > 0, v_v[j, 0:HALO, :], jnp.broadcast_to(row0[j], (HALO, 128)))

            def attend(a):
                for c in range(0, M, R):
                    o1, o2 = (_attend(q_v, k_v, v_v, r, r0 + (opaque(r, R) if OPQ[0] else r),
                                      opaque(r, R) if OPQ[1] else r, r0 + r if r < HALO else None)
                              for r in (a * T + c, a * T + M + c))
                    for j in range(hb):
                        for t, y in enumerate(_lhs_terms(o1[j], o1[j + hb], o2[j], o2[j + hb])):
                            o_v[a, t, c // 2:(c + R) // 2, 128 * j:128 * (j + 1)] = y

            def out_proj(a):
                n = D // 2 // NO
                for c0 in range(0, D // 2, n):
                    y = _strassen(lambda t: o_v[a, t], lambda t: wo_v[t, :, c0:c0 + n], (OO, OO1)[a])
                    for (ra, b), c in zip(QUADRANTS, y):
                        rr, cc = pl.ds(r0 + a * T + ra * M, M), pl.ds(b * (D // 2) + c0, n)
                        h_v[rr, cc] = x_v[rr, cc].astype(f32) + c

            steps = dict(q=lambda a: project(i * NH + a, wq_v, q_v, a * T, (OQ, OQ1)[a], NQ), v=values, a=attend, o=out_proj)
            for step in ORDER.split():
                steps[step[0]](int(step[1]))
            if PC:
                for which in (4, 5, 6):
                    w_ref = raw_v[which]
                    n = w_ref.shape[0] // 7 // na
                    for c in range(0, n, 16):
                        for c0 in range(0, w_ref.shape[1], PC):
                            _prepare_ffn(w_ref, pl.multiple_of(i * n, 16) + opaque(c, 16), c0,
                                         min(PC, w_ref.shape[1] - c0))

    with jax.named_scope("sc_5_ln"):
        @pl.loop(0, 2)
        def _(part):
            normalize(h_v, 0, part, 2)

    with jax.named_scope("sc_6_ffn"):
        @pl.loop(0, NT)
        def _(i):
            if not FFN:
                return
            for n, c in enumerate(range(0, F // 2 if FFN else FC, FC)):
                g = _strassen(lambda t: n_v[i, t], lambda t: _words(raw_v[4][t * (D // 2):(t + 1) * (D // 2), c:c + FC]), OG)
                u = _strassen(lambda t: n_v[i, t], lambda t: _words(raw_v[5][t * (D // 2):(t + 1) * (D // 2), c:c + FC]), OG)
                act = [jax.nn.gelu(a, approximate=True) * b for a, b in zip(g, u)]
                for t, a in enumerate(_lhs_terms(*act)):
                    act_v[t, :, c:c + FC] = a
            normalize_staggered(h_v, i + 1, LP2)
            y = _strassen(lambda t: act_v[t], lambda t: _words(raw_v[6][t * (F // 2):(t + 1) * (F // 2), :]), OD)
            for a in (1, 0):
                r = pl.multiple_of(i * T, T) + a * M
                for b in (0, 1):
                    cc = slice(b * (D // 2), (b + 1) * (D // 2))
                    out_v[pl.ds(r, M), cc] = (h_v[pl.ds(r, M), cc] + y[2 * a + b]).astype(bf16)
                if EARLY:
                    out_copy(r).start()
            if not EARLY:
                for a in (1, 0):
                    out_copy(pl.multiple_of(i * T, T) + a * M).start()

    with jax.named_scope("sc_7_out"):
        copy(out_v.at[0:S, :], out_hbm, osem).wait()


@jax.jit
def pallas_sequential_preLN__sliding_local_dilated__glu_gated_geglu__prompt_kernel(
        A_x, A_wqkv, A_wo, B_x, B_w_gate, B_w_up, B_w_down):
    del B_x
    any_spec = pl.BlockSpec(memory_space=pl.ANY)
    terms = lambda k, n: pltpu.VMEM((7, k // 4, n // 2), i32)
    na = NT // NH
    out = pl.pallas_call(
        _kernel,
        in_specs=[any_spec] * 6,
        out_specs=any_spec,
        out_shape=jax.ShapeDtypeStruct((S, D), bf16),
        scratch_shapes=[
            pltpu.VMEM((S + 16, D), bf16),
            [pltpu.VMEM((2, D // 2 + 16, D), bf16)] * 3 + [pltpu.VMEM((NB, 128, D), bf16)]
            + [pltpu.VMEM((7 * D // 2, F // 2), bf16)] * 2
            + [pltpu.VMEM((7 * F // 2, D // 2), bf16)],
            pltpu.VMEM((NT + 1, 7, M // 2, D // 2), i32),
            terms(D, D), terms(D, D), terms(D, D), terms(D, D),
            pltpu.VMEM((NB, NH * T, 128), f32), pltpu.VMEM((NB, S + HALO, 128), f32),
            pltpu.VMEM((NB, NH * T + HALO, 128), f32), pltpu.VMEM((NH, 7, M // 2, D // 2), i32),
            pltpu.VMEM((S + 8, D), f32), terms(T, F),
            pltpu.SemaphoreType.DMA((2,)), pltpu.SemaphoreType.DMA((4,)), pltpu.SemaphoreType.DMA((4,)),
            pltpu.SemaphoreType.DMA((2,)),
            pltpu.SemaphoreType.DMA,
        ],
        compiler_params=pltpu.CompilerParams(vmem_limit_bytes=120 * 1024 * 1024, flags=FLAGS, disable_bounds_checks=NOCHK),
    )(A_x.reshape(S, D), A_wqkv.reshape(2, D // 2, 3 * D), A_wo.reshape(NB, 128, D), B_w_gate, B_w_up, B_w_down)
    return out.reshape(1, S, D)
```

```python
import jax
import jax.numpy as jnp
import jax.experimental.pallas as pl
import jax.experimental.pallas.tpu as pltpu

S, D, F = 2048, 1024, 3584
HEAD_DIM, WINDOW, DILATION = 32, 8, 2
EPS = 1e-5
SCALE = HEAD_DIM ** -0.5
LOG2E = 1.4426950408889634

NB = D // 128
HB = NB // 2
HALO = 16
T = 256
M = T // 2
NT = S // T
NK = 4
NH = 2
NA = NT // NH
R = 32
FC = 256
PC = 512

K_PLAN = ("1304265", 2)
V_PLAN = ("1302546", 2)
Q_PLAN = (("1302564", 4), ("1304265", 4))
O_PLAN = (("2403651", 2), ("1304265", 2))
GATE_UP_ORDER = "1304265"
DOWN_ORDER = "1302546"

f32, bf16, i32 = jnp.float32, jnp.bfloat16, jnp.int32

QUADRANTS = ((0, 0), (0, 1), (1, 0), (1, 1))
SIGNS = ({0: 1, 3: 1, 4: -1, 6: 1}, {2: 1, 4: 1}, {1: 1, 3: 1}, {0: 1, 1: -1, 2: 1, 5: 1})


def _words(x):
    return pltpu.bitcast(x.astype(bf16), i32)


def _lhs_terms(a11, a12, a21, a22):
    return [_words(t) for t in (a11 + a22, a21 + a22, a11, a22, a11 + a12, a21 - a11, a12 - a22)]


def _rhs_terms(b11, b12, b21, b22):
    c11, c12, c21, c22 = (b.astype(f32) for b in (b11, b12, b21, b22))
    return [_words(t) for t in (c11 + c22, b11, c12 - c22, c21 - c11, b22, c11 + c12, c21 + c22)]


def _strassen(lhs, rhs, order):
    out = [None] * 4
    for i in map(int, order):
        m = jnp.dot(pltpu.bitcast(lhs(i), bf16), pltpu.bitcast(rhs(i), bf16), preferred_element_type=f32)
        for q, signs in enumerate(SIGNS):
            if i not in signs:
                continue
            if out[q] is None:
                out[q] = (m, signs[i])
            else:
                acc, sign = out[q]
                out[q] = (acc + m, sign) if sign == signs[i] else (acc - m, 1) if sign > 0 else (m - acc, 1)
    return [acc for acc, _ in out]


def _layernorm(x):
    c = x - jnp.mean(x, axis=-1, keepdims=True)
    return c * jax.lax.rsqrt(jnp.mean(c * c, axis=-1, keepdims=True) + EPS)


def _lane_xor(x, bits):
    lane = jax.lax.broadcasted_iota(i32, x.shape, 1)
    return jnp.take_along_axis(x, lane ^ bits, axis=1, mode="promise_in_bounds")


def _exchange_lanes(blocks):
    lane = jax.lax.broadcasted_iota(i32, blocks[0].shape, 1)
    blocks = [_lane_xor(b, 2 * j) if j else b for j, b in enumerate(blocks)]
    for t in (1, 2, 4):
        hi = (lane & (2 * t)) != 0
        blocks = [jnp.where(hi, blocks[j ^ t], blocks[j]) for j in range(NB)]
    return [_lane_xor(b, 2 * j) if j else b for j, b in enumerate(blocks)]


def _exchange_rows(blocks):
    row = jax.lax.broadcasted_iota(i32, blocks[0].shape, 0)
    for t in (1, 2, 4):
        hi = (row & t) != 0
        blocks = [jnp.where(hi, blocks[j], pltpu.roll(blocks[j ^ t], 8 - t, 0)) if j & t else
                  jnp.where(hi, pltpu.roll(blocks[j ^ t], t, 0), blocks[j]) for j in range(NB)]
    return blocks


def _prepare_qkv(raw, w_ref, r, n):
    k = n // 2
    blocks = _exchange_lanes([
        jnp.concatenate([_words(raw[a, pl.ds(r, n), 128 * j:128 * (j + 1)]) for a in (0, 1)])
        for j in range(NB)])
    for j in range(HB):
        quads = [pltpu.bitcast(blocks[j + b * HB][a * k:(a + 1) * k], bf16) for a, b in QUADRANTS]
        for i, t in enumerate(_rhs_terms(*quads)):
            w_ref[i, pl.ds(pl.multiple_of(r // 2, 8), k), 128 * j:128 * (j + 1)] = t


def _prepare_wo(raw, w_ref, m):
    for c in range(0, D // 2, 128):
        halves = []
        for c0 in (c, D // 2 + c):
            blocks = [_words(raw[j, pl.ds(pl.multiple_of(16 * m, 16), 16), c0:c0 + 128]) for j in range(NB)]
            halves.append([pltpu.bitcast(t, bf16) for t in _exchange_rows(blocks)])
        for j in range(HB):
            for i, t in enumerate(_rhs_terms(halves[0][j], halves[1][j], halves[0][j + HB], halves[1][j + HB])):
                w_ref[i, pl.ds(pl.multiple_of(64 * j + 8 * m, 8), 8), c:c + 128] = t


def _prepare_ffn(w_ref, r, c, n):
    at = lambda i: (pl.ds(i * (w_ref.shape[0] // 7) + r, 16), slice(c, c + n))
    terms = _rhs_terms(*(w_ref[at(i)] for i in (1, 2, 3, 4)))
    for i in (0, 2, 3, 5, 6):
        w_ref[at(i)] = pltpu.bitcast(terms[i], bf16)


def _sum(t):
    while len(t) > 1:
        t = [a + b for a, b in zip(t[::2], t[1::2])]
    return t[0]


def _attend(q_ref, k_ref, v_ref, r, pos, masked):
    window = lambda ref, j, r0, w: ref[j, pl.ds(r0 + HALO - DILATION * w, R), :]
    q = [q_ref[j, r:r + R, :] for j in range(NB)]
    logits = []
    for w in range(WINDOW):
        s = _sum([q[j] * window(k_ref, j, pos, w) for j in range(NB)])
        for b in (1, 16):
            s = s + _lane_xor(s, b)
        if masked and w:
            s = jnp.where(pos + jax.lax.broadcasted_iota(i32, s.shape, 0) >= DILATION * w, s, -1e9 / SCALE)
        logits.append(s)
    top = logits[0]
    for s in logits[1:]:
        top = jnp.maximum(top, s)
    e = [jnp.exp2((s - top) * (SCALE * LOG2E)) for s in logits]
    inv = 1.0 / _sum(e)
    p = [t * inv for t in e]
    return [_sum([p[w] * window(v_ref, j, r, w) for w in range(WINDOW)]) for j in range(NB)]


def _kernel(x_hbm, wqkv_hbm, wo_hbm, wg_hbm, wu_hbm, wd_hbm, out_hbm,
            x_v, qkv_raw, wo_raw, wg_v, wu_v, wd_v, n_v, wq_v, wk_v, wv_v, wo_v, q_v, k_v, v_v, o_v, h_v, act_v,
            wk_sem, w_sem, x_sem, ffn_sem, out_sem):
    out_v = x_v
    copy = pltpu.make_async_copy

    def rows(i, n):
        return pl.ds(i * n if isinstance(i, int) else pl.multiple_of(i * n, n), n)

    def qkv_slab(which, parts, i, sem):
        r = rows(i, D // 2 // parts)
        return copy(wqkv_hbm.at[:, r, which * D:(which + 1) * D], qkv_raw[which].at[:, r, :], sem)

    def x_rows(i, n, sem):
        return copy(x_hbm.at[rows(i, n), :], x_v.at[rows(i, n), :], sem)

    def wk_copies(i, step):
        sem = wk_sem.at[step % 2]
        return [qkv_slab(1, NK, i, sem), x_rows(i, M // NK, sem), x_rows(NK + i, M // NK, sem)]

    def w_copies(i, step):
        sem = w_sem.at[step % 4]
        return [qkv_slab(0, NT, i, sem), qkv_slab(2, NT, i, sem),
                copy(wo_hbm.at[:, rows(i, 16), :], wo_raw.at[:, rows(i, 16), :], sem)]

    def x_copies(i, step):
        return [x_rows(i, T, x_sem.at[step % 4])]

    def ffn_copies(i, step, halves=(0, 1)):
        out = []
        for src, dst in ((wg_hbm, wg_v), (wu_hbm, wu_v), (wd_hbm, wd_v)):
            n, nc = dst.shape[0] // 7 // NA, dst.shape[1]
            for a in halves:
                for b in (0, 1):
                    out.append(copy(src.at[rows(a * NA + i, n), b * nc:(b + 1) * nc],
                                    dst.at[rows((1 + 2 * a + b) * NA + i, n), :], ffn_sem.at[step % 2]))
        return out

    def start(copies, i, *args):
        for c in copies(i, i, *args):
            c.start()

    def wait(copies, i):
        for c in copies(0, i):
            c.wait()

    def opaque(c, n, salt):
        return pl.multiple_of(jnp.minimum(salt + c, c), n)

    def fence(ref, index, salt, words):
        value = pltpu.bitcast(words[-8:, -128:], ref.dtype)
        spare = ref.shape[-2] - value.shape[0]
        ref[(*index, pl.ds(opaque(spare, value.shape[0], salt), value.shape[0]), slice(0, 128))] = value

    def normalize(src, i, part, parts):
        n = M // parts
        top, bottom = (_layernorm(src[pl.ds(pl.multiple_of(i % NT * T + r + part * n, n), n), :].astype(f32))
                       for r in (0, M))
        terms = _lhs_terms(top[:, :D // 2], top[:, D // 2:], bottom[:, :D // 2], bottom[:, D // 2:])
        for t, a in enumerate(terms):
            n_v[i, t, rows(part, n // 2), :] = a
        return terms[-1]

    def normalize_staggered(src, i, parts):
        for part in range(parts):
            last = normalize(src, i, part, parts)
            fence(src, (), i + part, last)
        return last

    def project(i, w_ref, dst, r0, order, chunks):
        first, n = {}, HB // chunks
        for c0 in range(0, HB, n):
            y = _strassen(lambda t: n_v[i, t], lambda t: w_ref[t, :, 128 * c0:128 * (c0 + n)], order)
            for (a, b), c in zip(QUADRANTS, y):
                for j in range(n):
                    dst[b * HB + c0 + j, pl.ds(r0 + a * M, M), :] = c[:, 128 * j:128 * (j + 1)]
                    if a == 0:
                        first[b * HB + c0 + j] = c[0:1, 128 * j:128 * (j + 1)]
        return first

    start(wk_copies, 0)
    start(wk_copies, 1)

    @pl.loop(0, NK)
    def _(i):
        wait(wk_copies, i)

        @pl.when(i + 2 < NK)
        def _():
            start(wk_copies, i + 2)

        @pl.when(i + 2 == NK)
        def _():
            start(w_copies, 0)
            start(x_copies, 1)

        n = D // 2 // NK
        _prepare_qkv(qkv_raw[1], wk_v, pl.multiple_of(i * n, n), n)
        normalize(x_v, 0, i, NK)

    start(w_copies, 1)
    start(x_copies, 2)

    @pl.loop(0, NT)
    def _(i):
        @pl.when(i + 3 < NT)
        def _():
            start(x_copies, i + 3)

        @pl.when(i + 2 < NT)
        def _():
            start(w_copies, i + 2)

        for a in (0, 1):
            @pl.when(i == NT - 3 + a)
            def _():
                start(ffn_copies, 0, [a])

        @pl.when(i + 1 < NT)
        def _():
            wait(x_copies, i + 1)

        wait(w_copies, i)
        project(i, wk_v, k_v, pl.multiple_of(i * T, T) + HALO, *K_PLAN)
        n = D // 2 // NT
        _prepare_qkv(qkv_raw[0], wq_v, pl.multiple_of(i * n, n), n)
        last = normalize_staggered(x_v, i + 1, 2)
        for a in (0, 1):
            fence(qkv_raw[2], (a,), i, last)
        _prepare_qkv(qkv_raw[2], wv_v, pl.multiple_of(i * n, n), n)
        _prepare_wo(wo_raw, wo_v, i)

    for j in range(NB):
        k_v[j, 0:HALO, :] = jnp.broadcast_to(k_v[j, HALO:HALO + 1, :], (HALO, 128))
        v_v[j, NH * T:NH * T + HALO, :] = jnp.zeros((HALO, 128), f32)

    @pl.loop(0, NA)
    def _(i):
        for n in range(1, NA):
            @pl.when(i + 1 == n)
            def _():
                start(ffn_copies, n)

        wait(ffn_copies, i)
        r0 = pl.multiple_of(i * (NH * T), NH * T)
        v_v[:, 0:HALO, :] = v_v[:, NH * T:NH * T + HALO, :]
        first = project(i * NH, wv_v, v_v, HALO, *V_PLAN)
        for j in range(NB):
            v_v[j, 0:HALO, :] = jnp.where(i > 0, v_v[j, 0:HALO, :], jnp.broadcast_to(first[j], (HALO, 128)))
        for a in range(NH):
            project(i * NH + a, wq_v, q_v, a * T, *Q_PLAN[a])
        for a in range(1, NH):
            project(i * NH + a, wv_v, v_v, HALO + a * T, *V_PLAN)

        for a in range(NH):
            for c in range(0, M, R):
                top, bottom = (_attend(q_v, k_v, v_v, r, r0 + r, r < HALO) for r in (a * T + c, a * T + M + c))
                for j in range(HB):
                    for t, y in enumerate(_lhs_terms(top[j], top[j + HB], bottom[j], bottom[j + HB])):
                        o_v[a, t, c // 2:(c + R) // 2, 128 * j:128 * (j + 1)] = y

        for a, (order, chunks) in enumerate(O_PLAN):
            n = D // 2 // chunks
            for c0 in range(0, D // 2, n):
                y = _strassen(lambda t: o_v[a, t], lambda t: wo_v[t, :, c0:c0 + n], order)
                for (ra, b), c in zip(QUADRANTS, y):
                    rr, cc = pl.ds(r0 + a * T + ra * M, M), pl.ds(b * (D // 2) + c0, n)
                    h_v[rr, cc] = x_v[rr, cc].astype(f32) + c

        step = 0
        for w_ref in (wg_v, wu_v, wd_v):
            n = w_ref.shape[0] // 7 // NA
            for c in range(0, n, 16):
                for c0 in range(0, w_ref.shape[1], PC):
                    step += 1
                    _prepare_ffn(w_ref, pl.multiple_of(i * n, 16) + opaque(c, 16, i + step), c0,
                                 min(PC, w_ref.shape[1] - c0))

    @pl.loop(0, 2)
    def _(part):
        normalize(h_v, 0, part, 2)

    @pl.loop(0, NT)
    def _(i):
        for c in range(0, F // 2, FC):
            g, u = (_strassen(lambda t: n_v[i, t],
                              lambda t: _words(w_ref[t * (D // 2):(t + 1) * (D // 2), c:c + FC]), GATE_UP_ORDER)
                    for w_ref in (wg_v, wu_v))
            act = [jax.nn.gelu(a, approximate=True) * b for a, b in zip(g, u)]
            for t, a in enumerate(_lhs_terms(*act)):
                act_v[t, :, c:c + FC] = a
        normalize_staggered(h_v, i + 1, 8)
        y = _strassen(lambda t: act_v[t], lambda t: _words(wd_v[t * (F // 2):(t + 1) * (F // 2), :]), DOWN_ORDER)
        for a in (1, 0):
            rr = pl.ds(pl.multiple_of(i * T, T) + a * M, M)
            for b in (0, 1):
                cc = slice(b * (D // 2), (b + 1) * (D // 2))
                out_v[rr, cc] = (h_v[rr, cc] + y[2 * a + b]).astype(bf16)
            copy(out_v.at[rr, :], out_hbm.at[rr, :], out_sem).start()

    copy(out_v.at[0:S, :], out_hbm, out_sem).wait()


@jax.jit
def pallas_sequential_preLN__sliding_local_dilated__glu_gated_geglu__prompt_kernel(
    A_x: jax.Array,
    A_wqkv: jax.Array,
    A_wo: jax.Array,
    B_x: jax.Array,
    B_w_gate: jax.Array,
    B_w_up: jax.Array,
    B_w_down: jax.Array,
):
    del B_x
    vmem, sems = pltpu.VMEM, pltpu.SemaphoreType.DMA
    square = vmem((7, D // 4, D // 2), i32)
    any_spec = pl.BlockSpec(memory_space=pl.ANY)
    out = pl.pallas_call(
        _kernel,
        in_specs=[any_spec] * 6,
        out_specs=any_spec,
        out_shape=jax.ShapeDtypeStruct((S, D), bf16),
        scratch_shapes=[
            vmem((S + 16, D), bf16),
            [vmem((2, D // 2 + 16, D), bf16)] * 3,
            vmem((NB, 128, D), bf16),
            vmem((7 * D // 2, F // 2), bf16),
            vmem((7 * D // 2, F // 2), bf16),
            vmem((7 * F // 2, D // 2), bf16),
            vmem((NT + 1, 7, M // 2, D // 2), i32),
            square, square, square, square,
            vmem((NB, NH * T, 128), f32),
            vmem((NB, HALO + S, 128), f32),
            vmem((NB, HALO + NH * T, 128), f32),
            vmem((NH, 7, M // 2, D // 2), i32),
            vmem((S + 8, D), f32),
            vmem((7, M // 2, F // 2), i32),
            sems((2,)), sems((4,)), sems((4,)), sems((2,)), sems(()),
        ],
        compiler_params=pltpu.CompilerParams(vmem_limit_bytes=120 * 1024 * 1024),
    )(A_x.reshape(S, D), A_wqkv.reshape(2, D // 2, 3 * D), A_wo.reshape(NB, 128, D), B_w_gate, B_w_up, B_w_down)
    return out.reshape(1, S, D)
```

```python
import jax
import jax.numpy as jnp
import jax.experimental.pallas as pl
import jax.experimental.pallas.tpu as pltpu

S, D, F = 2048, 1024, 3584
HEAD_DIM, WINDOW, DILATION = 32, 8, 2
EPS = 1e-5
SCALE = HEAD_DIM ** -0.5
LOG2E = 1.4426950408889634

NB = D // 128
HB = NB // 2
HALO = 16
T = 256
M = T // 2
NT = S // T
NK = 4
NH = 2
NA = NT // NH
R = 64
FC = 256
PC = 512

ORDER = (1, 3, 0, 4, 2, 6, 5)
DOWN_ORDER = (1, 3, 0, 2, 5, 4, 6)

f32, bf16, i32 = jnp.float32, jnp.bfloat16, jnp.int32

QUADRANTS = ((0, 0), (0, 1), (1, 0), (1, 1))
SIGNS = ({0: 1, 3: 1, 4: -1, 6: 1}, {2: 1, 4: 1}, {1: 1, 3: 1}, {0: 1, 1: -1, 2: 1, 5: 1})


def _words(x):
    return pltpu.bitcast(x.astype(bf16), i32)


def _lhs_terms(a11, a12, a21, a22):
    return [_words(t) for t in (a11 + a22, a21 + a22, a11, a22, a11 + a12, a21 - a11, a12 - a22)]


def _rhs_terms(b11, b12, b21, b22):
    c11, c12, c21, c22 = (b.astype(f32) for b in (b11, b12, b21, b22))
    return [_words(t) for t in (c11 + c22, b11, c12 - c22, c21 - c11, b22, c11 + c12, c21 + c22)]


def _strassen(lhs, rhs, order=ORDER):
    out = [None] * 4
    for i in order:
        m = jnp.dot(pltpu.bitcast(lhs(i), bf16), pltpu.bitcast(rhs(i), bf16), preferred_element_type=f32)
        for q, signs in enumerate(SIGNS):
            if i not in signs:
                continue
            if out[q] is None:
                out[q] = (m, signs[i])
            else:
                acc, sign = out[q]
                out[q] = (acc + m, sign) if sign == signs[i] else (acc - m, 1) if sign > 0 else (m - acc, 1)
    return [acc for acc, _ in out]


def _layernorm(x):
    c = x - jnp.mean(x, axis=-1, keepdims=True)
    return c * jax.lax.rsqrt(jnp.mean(c * c, axis=-1, keepdims=True) + EPS)


def _lane_xor(x, bits):
    lane = jax.lax.broadcasted_iota(i32, x.shape, 1)
    return jnp.take_along_axis(x, lane ^ bits, axis=1, mode="promise_in_bounds")


def _exchange_lanes(blocks):
    lane = jax.lax.broadcasted_iota(i32, blocks[0].shape, 1)
    blocks = [_lane_xor(b, 2 * j) if j else b for j, b in enumerate(blocks)]
    for t in (1, 2, 4):
        hi = (lane & (2 * t)) != 0
        blocks = [jnp.where(hi, blocks[j ^ t], blocks[j]) for j in range(NB)]
    return [_lane_xor(b, 2 * j) if j else b for j, b in enumerate(blocks)]


def _exchange_rows(blocks):
    row = jax.lax.broadcasted_iota(i32, blocks[0].shape, 0)
    for t in (1, 2, 4):
        hi = (row & t) != 0
        blocks = [jnp.where(hi, blocks[j], pltpu.roll(blocks[j ^ t], 8 - t, 0)) if j & t else
                  jnp.where(hi, pltpu.roll(blocks[j ^ t], t, 0), blocks[j]) for j in range(NB)]
    return blocks


def _prepare_qkv(raw, w_ref, r, n):
    k = n // 2
    blocks = _exchange_lanes([
        jnp.concatenate([_words(raw[a, pl.ds(r, n), 128 * j:128 * (j + 1)]) for a in (0, 1)])
        for j in range(NB)])
    for j in range(HB):
        quads = [pltpu.bitcast(blocks[j + b * HB][a * k:(a + 1) * k], bf16) for a, b in QUADRANTS]
        for i, t in enumerate(_rhs_terms(*quads)):
            w_ref[i, pl.ds(pl.multiple_of(r // 2, 8), k), 128 * j:128 * (j + 1)] = t


def _prepare_wo(raw, w_ref, m):
    for c in range(0, D // 2, 128):
        halves = []
        for c0 in (c, D // 2 + c):
            blocks = [_words(raw[j, pl.ds(pl.multiple_of(16 * m, 16), 16), c0:c0 + 128]) for j in range(NB)]
            halves.append([pltpu.bitcast(t, bf16) for t in _exchange_rows(blocks)])
        for j in range(HB):
            for i, t in enumerate(_rhs_terms(halves[0][j], halves[1][j], halves[0][j + HB], halves[1][j + HB])):
                w_ref[i, pl.ds(pl.multiple_of(64 * j + 8 * m, 8), 8), c:c + 128] = t


def _prepare_ffn(w_ref, r, c, n):
    at = lambda i: (pl.ds(i * (w_ref.shape[0] // 7) + r, 16), slice(c, c + n))
    terms = _rhs_terms(*(w_ref[at(i)] for i in (1, 2, 3, 4)))
    for i in (0, 2, 3, 5, 6):
        w_ref[at(i)] = pltpu.bitcast(terms[i], bf16)


def _sum(t):
    while len(t) > 1:
        t = [a + b for a, b in zip(t[::2], t[1::2])]
    return t[0]


def _attend(q_ref, k_ref, v_ref, r, pos, masked):
    window = lambda ref, j, r0, w: ref[j, pl.ds(r0 + HALO - DILATION * w, R), :]
    q = [q_ref[j, r:r + R, :] for j in range(NB)]
    logits = []
    for w in range(WINDOW):
        s = _sum([q[j] * window(k_ref, j, pos, w) for j in range(NB)])
        for b in (1, 16):
            s = s + _lane_xor(s, b)
        if masked and w:
            s = jnp.where(pos + jax.lax.broadcasted_iota(i32, s.shape, 0) >= DILATION * w, s, -1e9 / SCALE)
        logits.append(s)
    top = logits[0]
    for s in logits[1:]:
        top = jnp.maximum(top, s)
    e = [jnp.exp2((s - top) * (SCALE * LOG2E)) for s in logits]
    inv = 1.0 / _sum(e)
    p = [t * inv for t in e]
    return [_sum([p[w] * window(v_ref, j, r, w) for w in range(WINDOW)]) for j in range(NB)]


def _kernel(x_hbm, wqkv_hbm, wo_hbm, wg_hbm, wu_hbm, wd_hbm, out_hbm,
            x_v, qkv_raw, wo_raw, wg_v, wu_v, wd_v, n_v, wq_v, wk_v, wv_v, wo_v, q_v, k_v, v_v, o_v, h_v, act_v,
            wk_sem, w_sem, x_sem, ffn_sem, out_sem):
    out_v = x_v
    copy = pltpu.make_async_copy

    def rows(i, n):
        return pl.ds(i * n if isinstance(i, int) else pl.multiple_of(i * n, n), n)

    def qkv_slab(which, parts, i, sem):
        r = rows(i, D // 2 // parts)
        return copy(wqkv_hbm.at[:, r, which * D:(which + 1) * D], qkv_raw[which].at[:, r, :], sem)

    def x_rows(i, n, sem):
        return copy(x_hbm.at[rows(i, n), :], x_v.at[rows(i, n), :], sem)

    def wk_copies(i, step):
        sem = wk_sem.at[step % 2]
        return [qkv_slab(1, NK, i, sem), x_rows(i, M // NK, sem), x_rows(NK + i, M // NK, sem)]

    def w_copies(i, step):
        sem = w_sem.at[step % 4]
        return [qkv_slab(0, NT, i, sem), qkv_slab(2, NT, i, sem),
                copy(wo_hbm.at[:, rows(i, 16), :], wo_raw.at[:, rows(i, 16), :], sem)]

    def x_copies(i, step):
        return [x_rows(i, T, x_sem.at[step % 4])]

    def ffn_copies(i, step, halves=(0, 1)):
        out = []
        for src, dst in ((wg_hbm, wg_v), (wu_hbm, wu_v), (wd_hbm, wd_v)):
            n, nc = dst.shape[0] // 7 // NA, dst.shape[1]
            for a in halves:
                for b in (0, 1):
                    out.append(copy(src.at[rows(a * NA + i, n), b * nc:(b + 1) * nc],
                                    dst.at[rows((1 + 2 * a + b) * NA + i, n), :], ffn_sem.at[step % 2]))
        return out

    def start(copies, i, *args):
        for c in copies(i, i, *args):
            c.start()

    def wait(copies, i):
        for c in copies(0, i):
            c.wait()

    def opaque(c, n, salt):
        return pl.multiple_of(jnp.minimum(salt + c, c), n)

    def fence(ref, index, salt, words):
        value = pltpu.bitcast(words[-8:, -128:], ref.dtype)
        spare = ref.shape[-2] - value.shape[0]
        ref[(*index, pl.ds(opaque(spare, value.shape[0], salt), value.shape[0]), slice(0, 128))] = value

    def normalize(src, i, part, parts):
        n = M // parts
        top, bottom = (_layernorm(src[rows((i % NT * 2 + a) * parts + part, n), :].astype(f32)) for a in (0, 1))
        terms = _lhs_terms(top[:, :D // 2], top[:, D // 2:], bottom[:, :D // 2], bottom[:, D // 2:])
        for t, a in enumerate(terms):
            n_v[i, t, rows(part, n // 2), :] = a
        return terms[-1]

    def normalize_staggered(src, i, parts):
        for part in range(parts):
            last = normalize(src, i, part, parts)
            fence(src, (), i + part, last)
        return last

    def project(i, w_ref, dst, r0, chunks):
        first, n = {}, HB // chunks
        for c0 in range(0, HB, n):
            y = _strassen(lambda t: n_v[i, t], lambda t: w_ref[t, :, 128 * c0:128 * (c0 + n)])
            for (a, b), c in zip(QUADRANTS, y):
                for j in range(n):
                    dst[b * HB + c0 + j, pl.ds(r0 + a * M, M), :] = c[:, 128 * j:128 * (j + 1)]
                    if a == 0:
                        first[b * HB + c0 + j] = c[0:1, 128 * j:128 * (j + 1)]
        return first

    start(wk_copies, 0)
    start(wk_copies, 1)

    @pl.loop(0, NK)
    def _(i):
        wait(wk_copies, i)

        @pl.when(i + 2 < NK)
        def _():
            start(wk_copies, i + 2)

        @pl.when(i + 2 == NK)
        def _():
            start(w_copies, 0)
            start(x_copies, 1)

        n = D // 2 // NK
        _prepare_qkv(qkv_raw[1], wk_v, pl.multiple_of(i * n, n), n)
        normalize(x_v, 0, i, NK)

    start(w_copies, 1)
    start(x_copies, 2)

    @pl.loop(0, NT)
    def _(i):
        @pl.when(i + 3 < NT)
        def _():
            start(x_copies, i + 3)

        @pl.when(i + 2 < NT)
        def _():
            start(w_copies, i + 2)

        for a in (0, 1):
            @pl.when(i == NT - 3 + a)
            def _():
                start(ffn_copies, 0, [a])

        @pl.when(i + 1 < NT)
        def _():
            wait(x_copies, i + 1)

        wait(w_copies, i)
        project(i, wk_v, k_v, pl.multiple_of(i * T, T) + HALO, 2)
        n = D // 2 // NT
        _prepare_qkv(qkv_raw[0], wq_v, pl.multiple_of(i * n, n), n)
        last = normalize_staggered(x_v, i + 1, 2)
        for a in (0, 1):
            fence(qkv_raw[2], (a,), i, last)
        _prepare_qkv(qkv_raw[2], wv_v, pl.multiple_of(i * n, n), n)
        _prepare_wo(wo_raw, wo_v, i)

    for j in range(NB):
        k_v[j, 0:HALO, :] = jnp.broadcast_to(k_v[j, HALO:HALO + 1, :], (HALO, 128))
        v_v[j, NH * T:NH * T + HALO, :] = jnp.zeros((HALO, 128), f32)

    @pl.loop(0, NA)
    def _(i):
        for n in range(1, NA):
            @pl.when(i + 1 == n)
            def _():
                start(ffn_copies, n)

        wait(ffn_copies, i)
        r0 = pl.multiple_of(i * (NH * T), NH * T)
        v_v[:, 0:HALO, :] = v_v[:, NH * T:NH * T + HALO, :]
        first = project(i * NH, wv_v, v_v, HALO, 2)
        for j in range(NB):
            v_v[j, 0:HALO, :] = jnp.where(i > 0, v_v[j, 0:HALO, :], jnp.broadcast_to(first[j], (HALO, 128)))
        for a in range(NH):
            project(i * NH + a, wq_v, q_v, a * T, 4)
        for a in range(1, NH):
            project(i * NH + a, wv_v, v_v, HALO + a * T, 2)

        for a in range(NH):
            for c in range(0, M, R):
                top, bottom = (_attend(q_v, k_v, v_v, r, r0 + r, r < HALO) for r in (a * T + c, a * T + M + c))
                for j in range(HB):
                    for t, y in enumerate(_lhs_terms(top[j], top[j + HB], bottom[j], bottom[j + HB])):
                        o_v[a, t, c // 2:(c + R) // 2, 128 * j:128 * (j + 1)] = y

        for a in range(NH):
            n = D // 4
            for c0 in range(0, D // 2, n):
                y = _strassen(lambda t: o_v[a, t], lambda t: wo_v[t, :, c0:c0 + n])
                for (ra, b), c in zip(QUADRANTS, y):
                    rr, cc = pl.ds(r0 + a * T + ra * M, M), pl.ds(b * (D // 2) + c0, n)
                    h_v[rr, cc] = x_v[rr, cc].astype(f32) + c

        step = 0
        for w_ref in (wg_v, wu_v, wd_v):
            n = w_ref.shape[0] // 7 // NA
            for c in range(0, n, 16):
                for c0 in range(0, w_ref.shape[1], PC):
                    step += 1
                    _prepare_ffn(w_ref, pl.multiple_of(i * n, 16) + opaque(c, 16, i + step), c0,
                                 min(PC, w_ref.shape[1] - c0))

    normalize(h_v, 0, 0, 1)

    @pl.loop(0, NT)
    def _(i):
        for c in range(0, F // 2, FC):
            g, u = (_strassen(lambda t: n_v[i, t],
                              lambda t: _words(w_ref[t * (D // 2):(t + 1) * (D // 2), c:c + FC]))
                    for w_ref in (wg_v, wu_v))
            act = [jax.nn.gelu(a, approximate=True) * b for a, b in zip(g, u)]
            for t, a in enumerate(_lhs_terms(*act)):
                act_v[t, :, c:c + FC] = a
        normalize_staggered(h_v, i + 1, 8)
        y = _strassen(lambda t: act_v[t], lambda t: _words(wd_v[t * (F // 2):(t + 1) * (F // 2), :]), DOWN_ORDER)
        for a in (1, 0):
            rr = pl.ds(pl.multiple_of(i * T, T) + a * M, M)
            for b in (0, 1):
                cc = slice(b * (D // 2), (b + 1) * (D // 2))
                out_v[rr, cc] = (h_v[rr, cc] + y[2 * a + b]).astype(bf16)
            copy(out_v.at[rr, :], out_hbm.at[rr, :], out_sem).start()

    copy(out_v.at[0:S, :], out_hbm, out_sem).wait()


@jax.jit
def pallas_sequential_preLN__sliding_local_dilated__glu_gated_geglu__prompt_kernel(
    A_x: jax.Array,
    A_wqkv: jax.Array,
    A_wo: jax.Array,
    B_x: jax.Array,
    B_w_gate: jax.Array,
    B_w_up: jax.Array,
    B_w_down: jax.Array,
):
    del B_x
    vmem, sems = pltpu.VMEM, pltpu.SemaphoreType.DMA
    square = vmem((7, D // 4, D // 2), i32)
    any_spec = pl.BlockSpec(memory_space=pl.ANY)
    out = pl.pallas_call(
        _kernel,
        in_specs=[any_spec] * 6,
        out_specs=any_spec,
        out_shape=jax.ShapeDtypeStruct((S, D), bf16),
        scratch_shapes=[
            vmem((S + 16, D), bf16),
            [vmem((2, D // 2 + 16, D), bf16)] * 3,
            vmem((NB, 128, D), bf16),
            vmem((7 * D // 2, F // 2), bf16),
            vmem((7 * D // 2, F // 2), bf16),
            vmem((7 * F // 2, D // 2), bf16),
            vmem((NT + 1, 7, M // 2, D // 2), i32),
            square, square, square, square,
            vmem((NB, NH * T, 128), f32),
            vmem((NB, HALO + S, 128), f32),
            vmem((NB, HALO + NH * T, 128), f32),
            vmem((NH, 7, M // 2, D // 2), i32),
            vmem((S + 8, D), f32),
            vmem((7, M // 2, F // 2), i32),
            sems((2,)), sems((4,)), sems((4,)), sems((2,)), sems(()),
        ],
        compiler_params=pltpu.CompilerParams(vmem_limit_bytes=120 * 1024 * 1024),
    )(A_x.reshape(S, D), A_wqkv.reshape(2, D // 2, 3 * D), A_wo.reshape(NB, 128, D), B_w_gate, B_w_up, B_w_down)
    return out.reshape(1, S, D)
```

```python
import jax
import jax.numpy as jnp
import jax.experimental.pallas as pl
import jax.experimental.pallas.tpu as pltpu

S, D, F = 2048, 1024, 3584
HEAD_DIM, WINDOW, DILATION = 32, 8, 2
EPS = 1e-5
SCALE = HEAD_DIM ** -0.5
LOG2E = 1.4426950408889634

NB = D // 128
HB = NB // 2
HALO = 16
T = 256
M = T // 2
NT = S // T
NK = 4
NH = 2
NA = NT // NH
FC = 256
PC = 256

ORDER = (1, 3, 0, 4, 2, 6, 5)
DOWN_ORDER = (1, 3, 0, 2, 5, 4, 6)

f32, bf16, i32 = jnp.float32, jnp.bfloat16, jnp.int32

QUADRANTS = ((0, 0), (0, 1), (1, 0), (1, 1))
SIGNS = ({0: 1, 3: 1, 4: -1, 6: 1}, {2: 1, 4: 1}, {1: 1, 3: 1}, {0: 1, 1: -1, 2: 1, 5: 1})


def _words(x):
    return pltpu.bitcast(x.astype(bf16), i32)


def _lhs_terms(a11, a12, a21, a22):
    return [_words(t) for t in (a11 + a22, a21 + a22, a11, a22, a11 + a12, a21 - a11, a12 - a22)]


def _rhs_terms(b11, b12, b21, b22):
    c11, c12, c21, c22 = (b.astype(f32) for b in (b11, b12, b21, b22))
    return [_words(t) for t in (c11 + c22, b11, c12 - c22, c21 - c11, b22, c11 + c12, c21 + c22)]


def _strassen(lhs, rhs, order=ORDER):
    out = [None] * 4
    for i in order:
        m = jnp.dot(pltpu.bitcast(lhs(i), bf16), pltpu.bitcast(rhs(i), bf16), preferred_element_type=f32)
        for q, signs in enumerate(SIGNS):
            if i not in signs:
                continue
            if out[q] is None:
                out[q] = (m, signs[i])
            else:
                acc, sign = out[q]
                out[q] = (acc + m, sign) if sign == signs[i] else (acc - m, 1) if sign > 0 else (m - acc, 1)
    return [acc for acc, _ in out]


def _layernorm(x):
    c = x - jnp.mean(x, axis=-1, keepdims=True)
    return c * jax.lax.rsqrt(jnp.mean(c * c, axis=-1, keepdims=True) + EPS)


def _lane_xor(x, bits):
    lane = jax.lax.broadcasted_iota(i32, x.shape, 1)
    return jnp.take_along_axis(x, lane ^ bits, axis=1, mode="promise_in_bounds")


def _exchange_lanes(blocks):
    lane = jax.lax.broadcasted_iota(i32, blocks[0].shape, 1)
    blocks = [_lane_xor(b, 2 * j) if j else b for j, b in enumerate(blocks)]
    for t in (1, 2, 4):
        hi = (lane & (2 * t)) != 0
        blocks = [jnp.where(hi, blocks[j ^ t], blocks[j]) for j in range(NB)]
    return [_lane_xor(b, 2 * j) if j else b for j, b in enumerate(blocks)]


def _exchange_rows(blocks):
    row = jax.lax.broadcasted_iota(i32, blocks[0].shape, 0)
    for t in (1, 2, 4):
        hi = (row & t) != 0
        blocks = [jnp.where(hi, blocks[j], pltpu.roll(blocks[j ^ t], 8 - t, 0)) if j & t else
                  jnp.where(hi, pltpu.roll(blocks[j ^ t], t, 0), blocks[j]) for j in range(NB)]
    return blocks


def _prepare_qkv(raw, w_ref, r, n):
    k = n // 2
    blocks = _exchange_lanes([
        jnp.concatenate([_words(raw[a, pl.ds(r, n), 128 * j:128 * (j + 1)]) for a in (0, 1)])
        for j in range(NB)])
    for j in range(HB):
        quads = [pltpu.bitcast(blocks[j + b * HB][a * k:(a + 1) * k], bf16) for a, b in QUADRANTS]
        for i, t in enumerate(_rhs_terms(*quads)):
            w_ref[i, pl.ds(pl.multiple_of(r // 2, 8), k), 128 * j:128 * (j + 1)] = t


def _prepare_wo(raw, w_ref, m):
    for c in range(0, D // 2, 128):
        halves = []
        for c0 in (c, D // 2 + c):
            blocks = [_words(raw[j, pl.ds(pl.multiple_of(16 * m, 16), 16), c0:c0 + 128]) for j in range(NB)]
            halves.append([pltpu.bitcast(t, bf16) for t in _exchange_rows(blocks)])
        for j in range(HB):
            for i, t in enumerate(_rhs_terms(halves[0][j], halves[1][j], halves[0][j + HB], halves[1][j + HB])):
                w_ref[i, pl.ds(pl.multiple_of(64 * j + 8 * m, 8), 8), c:c + 128] = t


def _prepare_ffn(w_ref, r, c, n):
    at = lambda i: (pl.ds(i * (w_ref.shape[0] // 7) + r, 16), slice(c, c + n))
    terms = _rhs_terms(*(w_ref[at(i)] for i in (1, 2, 3, 4)))
    for i in (0, 2, 3, 5, 6):
        w_ref[at(i)] = pltpu.bitcast(terms[i], bf16)


def _sum(t):
    while len(t) > 1:
        t = [a + b for a, b in zip(t[::2], t[1::2])]
    return t[0]


def _attend(q_ref, k_ref, v_ref, r, pos, masked):
    window = lambda ref, j, r0, w: ref[j, pl.ds(r0 + HALO - DILATION * w, M), :]
    q = [q_ref[j, r:r + M, :] for j in range(NB)]
    logits = []
    for w in range(WINDOW):
        s = _sum([q[j] * window(k_ref, j, pos, w) for j in range(NB)])
        for b in (1, 16):
            s = s + _lane_xor(s, b)
        if masked and w:
            s = jnp.where(pos + jax.lax.broadcasted_iota(i32, s.shape, 0) >= DILATION * w, s, -1e9 / SCALE)
        logits.append(s)
    top = logits[0]
    for s in logits[1:]:
        top = jnp.maximum(top, s)
    e = [jnp.exp2((s - top) * (SCALE * LOG2E)) for s in logits]
    inv = 1.0 / _sum(e)
    p = [t * inv for t in e]
    return [_sum([p[w] * window(v_ref, j, r, w) for w in range(WINDOW)]) for j in range(NB)]


def _kernel(x_hbm, wqkv_hbm, wo_hbm, wg_hbm, wu_hbm, wd_hbm, out_hbm,
            x_v, qkv_raw, wo_raw, wg_v, wu_v, wd_v, n_v, wq_v, wk_v, wv_v, wo_v, q_v, k_v, v_v, o_v, h_v, act_v,
            wk_sem, w_sem, x_sem, ffn_sem, out_sem):
    out_v = x_v
    copy = pltpu.make_async_copy

    def rows(i, n):
        return pl.ds(i * n if isinstance(i, int) else pl.multiple_of(i * n, n), n)

    def qkv_slab(which, parts, i, sem):
        r = rows(i, D // 2 // parts)
        return copy(wqkv_hbm.at[:, r, which * D:(which + 1) * D], qkv_raw[which].at[:, r, :], sem)

    def x_rows(i, n, sem):
        return copy(x_hbm.at[rows(i, n), :], x_v.at[rows(i, n), :], sem)

    def wk_copies(i, step):
        sem = wk_sem.at[step % 2]
        return [qkv_slab(1, NK, i, sem), x_rows(i, M // NK, sem), x_rows(NK + i, M // NK, sem)]

    def w_copies(i, step):
        sem = w_sem.at[step % 4]
        return [qkv_slab(0, NT, i, sem), qkv_slab(2, NT, i, sem),
                copy(wo_hbm.at[:, rows(i, 16), :], wo_raw.at[:, rows(i, 16), :], sem)]

    def x_copies(i, step):
        return [x_rows(i, T, x_sem.at[step % 4])]

    def ffn_copies(i, step, halves=(0, 1)):
        out = []
        for src, dst in ((wg_hbm, wg_v), (wu_hbm, wu_v), (wd_hbm, wd_v)):
            n, nc = dst.shape[0] // 7 // NA, dst.shape[1]
            for a in halves:
                for b in (0, 1):
                    out.append(copy(src.at[rows(a * NA + i, n), b * nc:(b + 1) * nc],
                                    dst.at[rows((1 + 2 * a + b) * NA + i, n), :], ffn_sem.at[step % 2]))
        return out

    def start(copies, i, *args):
        for c in copies(i, i, *args):
            c.start()

    def wait(copies, i):
        for c in copies(0, i):
            c.wait()

    def opaque(c, n, salt):
        return pl.multiple_of(jnp.minimum(salt + c, c), n)

    def normalize(src, i, part, parts):
        n = M // parts
        top, bottom = (_layernorm(src[rows((i % NT * 2 + a) * parts + part, n), :].astype(f32)) for a in (0, 1))
        terms = _lhs_terms(top[:, :D // 2], top[:, D // 2:], bottom[:, :D // 2], bottom[:, D // 2:])
        for t, a in enumerate(terms):
            n_v[i, t, rows(part, n // 2), :] = a
        return terms[-1]

    def normalize_staggered(src, i, parts):
        for part in range(parts):
            last = pltpu.bitcast(normalize(src, i, part, parts)[-8:, -128:], src.dtype)
            src[pl.ds(opaque(S, last.shape[0], i + part), last.shape[0]), 0:128] = last

    def project(i, w_ref, dst, r0, chunks):
        first, n = {}, HB // chunks
        for c0 in range(0, HB, n):
            y = _strassen(lambda t: n_v[i, t], lambda t: w_ref[t, :, 128 * c0:128 * (c0 + n)])
            for (a, b), c in zip(QUADRANTS, y):
                for j in range(n):
                    dst[b * HB + c0 + j, pl.ds(r0 + a * M, M), :] = c[:, 128 * j:128 * (j + 1)]
                    if a == 0:
                        first[b * HB + c0 + j] = c[0:1, 128 * j:128 * (j + 1)]
        return first

    start(wk_copies, 0)
    start(wk_copies, 1)

    @pl.loop(0, NK)
    def _(i):
        wait(wk_copies, i)

        @pl.when(i + 2 < NK)
        def _():
            start(wk_copies, i + 2)

        @pl.when(i + 2 == NK)
        def _():
            start(w_copies, 0)
            start(x_copies, 1)

        n = D // 2 // NK
        _prepare_qkv(qkv_raw[1], wk_v, pl.multiple_of(i * n, n), n)
        normalize(x_v, 0, i, NK)

    start(w_copies, 1)
    start(x_copies, 2)

    @pl.loop(0, NT)
    def _(i):
        @pl.when(i + 3 < NT)
        def _():
            start(x_copies, i + 3)

        @pl.when(i + 2 < NT)
        def _():
            start(w_copies, i + 2)

        for a in (0, 1):
            @pl.when(i == NT - 3 + a)
            def _():
                start(ffn_copies, 0, [a])

        @pl.when(i + 1 < NT)
        def _():
            wait(x_copies, i + 1)

        wait(w_copies, i)
        project(i, wk_v, k_v, pl.multiple_of(i * T, T) + HALO, 1)
        normalize_staggered(x_v, i + 1, 2)
        n = D // 2 // NT
        _prepare_qkv(qkv_raw[0], wq_v, pl.multiple_of(i * n, n), n)
        _prepare_qkv(qkv_raw[2], wv_v, pl.multiple_of(i * n, n), n)
        _prepare_wo(wo_raw, wo_v, i)

    for j in range(NB):
        k_v[j, 0:HALO, :] = jnp.broadcast_to(k_v[j, HALO:HALO + 1, :], (HALO, 128))
        v_v[j, NH * T:NH * T + HALO, :] = jnp.zeros((HALO, 128), f32)

    @pl.loop(0, NA)
    def _(i):
        for n in range(1, NA):
            @pl.when(i + 1 == n)
            def _():
                start(ffn_copies, n)

        wait(ffn_copies, i)
        r0 = pl.multiple_of(i * (NH * T), NH * T)
        v_v[:, 0:HALO, :] = v_v[:, NH * T:NH * T + HALO, :]
        first = project(i * NH, wv_v, v_v, HALO, 2)
        for j in range(NB):
            v_v[j, 0:HALO, :] = jnp.where(i > 0, v_v[j, 0:HALO, :], jnp.broadcast_to(first[j], (HALO, 128)))
        for a in range(NH):
            project(i * NH + a, wq_v, q_v, a * T, 4)
        for a in range(1, NH):
            project(i * NH + a, wv_v, v_v, HALO + a * T, 2)

        for a in range(NH):
            top, bottom = (_attend(q_v, k_v, v_v, r, r0 + r, r < HALO) for r in (a * T, a * T + M))
            for j in range(HB):
                for t, y in enumerate(_lhs_terms(top[j], top[j + HB], bottom[j], bottom[j + HB])):
                    o_v[a, t, :, 128 * j:128 * (j + 1)] = y

        for a in range(NH):
            n = D // 4
            for c0 in range(0, D // 2, n):
                y = _strassen(lambda t: o_v[a, t], lambda t: wo_v[t, :, c0:c0 + n])
                for (ra, b), c in zip(QUADRANTS, y):
                    rr, cc = pl.ds(r0 + a * T + ra * M, M), pl.ds(b * (D // 2) + c0, n)
                    h_v[rr, cc] = x_v[rr, cc].astype(f32) + c

        step = 0
        for w_ref in (wg_v, wu_v, wd_v):
            n = w_ref.shape[0] // 7 // NA
            for c in range(0, n, 16):
                for c0 in range(0, w_ref.shape[1], PC):
                    step += 1
                    _prepare_ffn(w_ref, pl.multiple_of(i * n, 16) + opaque(c, 16, i + step), c0, PC)

    normalize(h_v, 0, 0, 1)

    @pl.loop(0, NT)
    def _(i):
        for c in range(0, F // 2, FC):
            g, u = (_strassen(lambda t: n_v[i, t],
                              lambda t: _words(w_ref[t * (D // 2):(t + 1) * (D // 2), c:c + FC]))
                    for w_ref in (wg_v, wu_v))
            act = [jax.nn.gelu(a, approximate=True) * b for a, b in zip(g, u)]
            for t, a in enumerate(_lhs_terms(*act)):
                act_v[t, :, c:c + FC] = a
        normalize_staggered(h_v, i + 1, 8)
        y = _strassen(lambda t: act_v[t], lambda t: _words(wd_v[t * (F // 2):(t + 1) * (F // 2), :]), DOWN_ORDER)
        for a in (1, 0):
            rr = pl.ds(pl.multiple_of(i * T, T) + a * M, M)
            for b in (0, 1):
                cc = slice(b * (D // 2), (b + 1) * (D // 2))
                out_v[rr, cc] = (h_v[rr, cc] + y[2 * a + b]).astype(bf16)
            copy(out_v.at[rr, :], out_hbm.at[rr, :], out_sem).start()

    copy(out_v.at[0:S, :], out_hbm, out_sem).wait()


@jax.jit
def pallas_sequential_preLN__sliding_local_dilated__glu_gated_geglu__prompt_kernel(
    A_x: jax.Array,
    A_wqkv: jax.Array,
    A_wo: jax.Array,
    B_x: jax.Array,
    B_w_gate: jax.Array,
    B_w_up: jax.Array,
    B_w_down: jax.Array,
):
    del B_x
    vmem, sems = pltpu.VMEM, pltpu.SemaphoreType.DMA
    square = vmem((7, D // 4, D // 2), i32)
    any_spec = pl.BlockSpec(memory_space=pl.ANY)
    out = pl.pallas_call(
        _kernel,
        in_specs=[any_spec] * 6,
        out_specs=any_spec,
        out_shape=jax.ShapeDtypeStruct((S, D), bf16),
        scratch_shapes=[
            vmem((S + 16, D), bf16),
            [vmem((2, D // 2, D), bf16)] * 3,
            vmem((NB, 128, D), bf16),
            vmem((7 * D // 2, F // 2), bf16),
            vmem((7 * D // 2, F // 2), bf16),
            vmem((7 * F // 2, D // 2), bf16),
            vmem((NT + 1, 7, M // 2, D // 2), i32),
            square, square, square, square,
            vmem((NB, NH * T, 128), f32),
            vmem((NB, HALO + S, 128), f32),
            vmem((NB, HALO + NH * T, 128), f32),
            vmem((NH, 7, M // 2, D // 2), i32),
            vmem((S + 8, D), f32),
            vmem((7, M // 2, F // 2), i32),
            sems((2,)), sems((4,)), sems((4,)), sems((2,)), sems(()),
        ],
        compiler_params=pltpu.CompilerParams(
            vmem_limit_bytes=120 * 1024 * 1024,
            flags={"XLA_TPU_EVENLY_DISTRIBUTE_CRITICAL_NODES": True},
        ),
    )(A_x.reshape(S, D), A_wqkv.reshape(2, D // 2, 3 * D), A_wo.reshape(NB, 128, D), B_w_gate, B_w_up, B_w_down)
    return out.reshape(1, S, D)
```

```python
import jax
import jax.numpy as jnp
import jax.experimental.pallas as pl
import jax.experimental.pallas.tpu as pltpu

S, D, F = 2048, 1024, 3584
HEAD_DIM, WINDOW, DILATION = 32, 8, 2
EPS = 1e-5
SCALE = HEAD_DIM ** -0.5
LOG2E = 1.4426950408889634

NB = D // 128
HB = NB // 2
HALO = 16
T = 256
M = T // 2
NT = S // T
NK = 4
NH = 2
NA = NT // NH
FC = 256
PC = 256

ORDER = (1, 3, 0, 4, 2, 6, 5)
DOWN_ORDER = (1, 3, 0, 2, 5, 4, 6)

f32, bf16, i32 = jnp.float32, jnp.bfloat16, jnp.int32

QUADRANTS = ((0, 0), (0, 1), (1, 0), (1, 1))
SIGNS = ({0: 1, 3: 1, 4: -1, 6: 1}, {2: 1, 4: 1}, {1: 1, 3: 1}, {0: 1, 1: -1, 2: 1, 5: 1})


def _words(x):
    return pltpu.bitcast(x.astype(bf16), i32)


def _lhs_terms(a11, a12, a21, a22):
    return [_words(t) for t in (a11 + a22, a21 + a22, a11, a22, a11 + a12, a21 - a11, a12 - a22)]


def _rhs_terms(b11, b12, b21, b22):
    c11, c12, c21, c22 = (b.astype(f32) for b in (b11, b12, b21, b22))
    return [_words(t) for t in (c11 + c22, b11, c12 - c22, c21 - c11, b22, c11 + c12, c21 + c22)]


def _strassen(lhs, rhs, order=ORDER):
    out = [None] * 4
    for i in order:
        m = jnp.dot(pltpu.bitcast(lhs(i), bf16), pltpu.bitcast(rhs(i), bf16), preferred_element_type=f32)
        for q, signs in enumerate(SIGNS):
            if i not in signs:
                continue
            if out[q] is None:
                out[q] = (m, signs[i])
            else:
                acc, sign = out[q]
                out[q] = (acc + m, sign) if sign == signs[i] else (acc - m, 1) if sign > 0 else (m - acc, 1)
    return [acc for acc, _ in out]


def _layernorm(x):
    c = x - jnp.mean(x, axis=-1, keepdims=True)
    return c * jax.lax.rsqrt(jnp.mean(c * c, axis=-1, keepdims=True) + EPS)


def _lane_xor(x, bits):
    lane = jax.lax.broadcasted_iota(i32, x.shape, 1)
    return jnp.take_along_axis(x, lane ^ bits, axis=1, mode="promise_in_bounds")


def _exchange_lanes(blocks):
    lane = jax.lax.broadcasted_iota(i32, blocks[0].shape, 1)
    blocks = [_lane_xor(b, 2 * j) if j else b for j, b in enumerate(blocks)]
    for t in (1, 2, 4):
        hi = (lane & (2 * t)) != 0
        blocks = [jnp.where(hi, blocks[j ^ t], blocks[j]) for j in range(NB)]
    return [_lane_xor(b, 2 * j) if j else b for j, b in enumerate(blocks)]


def _exchange_rows(blocks):
    row = jax.lax.broadcasted_iota(i32, blocks[0].shape, 0)
    for t in (1, 2, 4):
        hi = (row & t) != 0
        blocks = [jnp.where(hi, blocks[j], pltpu.roll(blocks[j ^ t], 8 - t, 0)) if j & t else
                  jnp.where(hi, pltpu.roll(blocks[j ^ t], t, 0), blocks[j]) for j in range(NB)]
    return blocks


def _prepare_qkv(raw, w_ref, r, n):
    k = n // 2
    blocks = _exchange_lanes([
        jnp.concatenate([_words(raw[a, pl.ds(r, n), 128 * j:128 * (j + 1)]) for a in (0, 1)])
        for j in range(NB)])
    for j in range(HB):
        quads = [pltpu.bitcast(blocks[j + b * HB][a * k:(a + 1) * k], bf16) for a, b in QUADRANTS]
        for i, t in enumerate(_rhs_terms(*quads)):
            w_ref[i, pl.ds(pl.multiple_of(r // 2, 8), k), 128 * j:128 * (j + 1)] = t


def _prepare_wo(raw, w_ref, m):
    for c in range(0, D // 2, 128):
        halves = []
        for c0 in (c, D // 2 + c):
            blocks = [_words(raw[j, pl.ds(pl.multiple_of(16 * m, 16), 16), c0:c0 + 128]) for j in range(NB)]
            halves.append([pltpu.bitcast(t, bf16) for t in _exchange_rows(blocks)])
        for j in range(HB):
            for i, t in enumerate(_rhs_terms(halves[0][j], halves[1][j], halves[0][j + HB], halves[1][j + HB])):
                w_ref[i, pl.ds(pl.multiple_of(64 * j + 8 * m, 8), 8), c:c + 128] = t


def _prepare_ffn(w_ref, r, c, n):
    at = lambda i: (pl.ds(i * (w_ref.shape[0] // 7) + r, 16), slice(c, c + n))
    terms = _rhs_terms(*(w_ref[at(i)] for i in (1, 2, 3, 4)))
    for i in (0, 2, 3, 5, 6):
        w_ref[at(i)] = pltpu.bitcast(terms[i], bf16)


def _sum(t):
    while len(t) > 1:
        t = [a + b for a, b in zip(t[::2], t[1::2])]
    return t[0]


def _attend(q_ref, k_ref, v_ref, r, pos, masked):
    window = lambda ref, j, r0, w: ref[j, pl.ds(r0 + HALO - DILATION * w, M), :]
    q = [q_ref[j, r:r + M, :] for j in range(NB)]
    logits = []
    for w in range(WINDOW):
        s = _sum([q[j] * window(k_ref, j, pos, w) for j in range(NB)])
        for b in (1, 16):
            s = s + _lane_xor(s, b)
        if masked and w:
            s = jnp.where(pos + jax.lax.broadcasted_iota(i32, s.shape, 0) >= DILATION * w, s, -1e9 / SCALE)
        logits.append(s)
    top = logits[0]
    for s in logits[1:]:
        top = jnp.maximum(top, s)
    e = [jnp.exp2((s - top) * (SCALE * LOG2E)) for s in logits]
    inv = 1.0 / _sum(e)
    p = [t * inv for t in e]
    return [_sum([p[w] * window(v_ref, j, r, w) for w in range(WINDOW)]) for j in range(NB)]


def _kernel(x_hbm, wqkv_hbm, wo_hbm, wg_hbm, wu_hbm, wd_hbm, out_hbm,
            x_v, qkv_raw, wo_raw, wg_v, wu_v, wd_v, n_v, wq_v, wk_v, wv_v, wo_v, q_v, k_v, v_v, o_v, h_v, act_v,
            wk_sem, w_sem, x_sem, ffn_sem, out_sem):
    out_v = x_v
    copy = pltpu.make_async_copy

    def rows(i, n):
        return pl.ds(i * n if isinstance(i, int) else pl.multiple_of(i * n, n), n)

    def qkv_slab(which, parts, i, sem):
        r = rows(i, D // 2 // parts)
        return copy(wqkv_hbm.at[:, r, which * D:(which + 1) * D], qkv_raw[which].at[:, r, :], sem)

    def x_rows(i, n, sem):
        return copy(x_hbm.at[rows(i, n), :], x_v.at[rows(i, n), :], sem)

    def wk_copies(i, step):
        sem = wk_sem.at[step % 2]
        return [qkv_slab(1, NK, i, sem), x_rows(i, M // NK, sem), x_rows(NK + i, M // NK, sem)]

    def w_copies(i, step):
        sem = w_sem.at[step % 4]
        return [qkv_slab(0, NT, i, sem), qkv_slab(2, NT, i, sem),
                copy(wo_hbm.at[:, rows(i, 16), :], wo_raw.at[:, rows(i, 16), :], sem)]

    def x_copies(i, step):
        return [x_rows(i, T, x_sem.at[step % 4])]

    def ffn_copies(i, step, halves=(0, 1)):
        out = []
        for src, dst in ((wg_hbm, wg_v), (wu_hbm, wu_v), (wd_hbm, wd_v)):
            n, nc = dst.shape[0] // 7 // NA, dst.shape[1]
            for a in halves:
                for b in (0, 1):
                    out.append(copy(src.at[rows(a * NA + i, n), b * nc:(b + 1) * nc],
                                    dst.at[rows((1 + 2 * a + b) * NA + i, n), :], ffn_sem.at[step % 2]))
        return out

    def start(copies, i, *args):
        for c in copies(i, i, *args):
            c.start()

    def wait(copies, i):
        for c in copies(0, i):
            c.wait()

    def opaque(c, n, salt):
        return pl.multiple_of(jnp.minimum(salt + c, c), n)

    def normalize(src, i, part, parts):
        n = M // parts
        top, bottom = (_layernorm(src[rows((i % NT * 2 + a) * parts + part, n), :].astype(f32)) for a in (0, 1))
        terms = _lhs_terms(top[:, :D // 2], top[:, D // 2:], bottom[:, :D // 2], bottom[:, D // 2:])
        for t, a in enumerate(terms):
            n_v[i, t, rows(part, n // 2), :] = a
        return terms[-1]

    def project(i, w_ref, dst, r0, chunks):
        first, n = {}, HB // chunks
        for c0 in range(0, HB, n):
            y = _strassen(lambda t: n_v[i, t], lambda t: w_ref[t, :, 128 * c0:128 * (c0 + n)])
            for (a, b), c in zip(QUADRANTS, y):
                for j in range(n):
                    dst[b * HB + c0 + j, pl.ds(r0 + a * M, M), :] = c[:, 128 * j:128 * (j + 1)]
                    if a == 0:
                        first[b * HB + c0 + j] = c[0:1, 128 * j:128 * (j + 1)]
        return first

    start(wk_copies, 0)
    start(wk_copies, 1)

    @pl.loop(0, NK)
    def _(i):
        wait(wk_copies, i)

        @pl.when(i + 2 < NK)
        def _():
            start(wk_copies, i + 2)

        @pl.when(i + 2 == NK)
        def _():
            start(w_copies, 0)
            start(x_copies, 1)

        n = D // 2 // NK
        _prepare_qkv(qkv_raw[1], wk_v, pl.multiple_of(i * n, n), n)
        normalize(x_v, 0, i, NK)

    start(w_copies, 1)
    start(x_copies, 2)

    @pl.loop(0, NT)
    def _(i):
        @pl.when(i + 3 < NT)
        def _():
            start(x_copies, i + 3)

        @pl.when(i + 2 < NT)
        def _():
            start(w_copies, i + 2)

        for a in (0, 1):
            @pl.when(i == NT - 3 + a)
            def _():
                start(ffn_copies, 0, [a])

        @pl.when(i + 1 < NT)
        def _():
            wait(x_copies, i + 1)

        wait(w_copies, i)
        project(i, wk_v, k_v, pl.multiple_of(i * T, T) + HALO, 1)
        normalize(x_v, i + 1, 0, 1)
        n = D // 2 // NT
        _prepare_qkv(qkv_raw[0], wq_v, pl.multiple_of(i * n, n), n)
        _prepare_qkv(qkv_raw[2], wv_v, pl.multiple_of(i * n, n), n)
        _prepare_wo(wo_raw, wo_v, i)

    for j in range(NB):
        k_v[j, 0:HALO, :] = jnp.broadcast_to(k_v[j, HALO:HALO + 1, :], (HALO, 128))
        v_v[j, NH * T:NH * T + HALO, :] = jnp.zeros((HALO, 128), f32)

    @pl.loop(0, NA)
    def _(i):
        for n in range(1, NA):
            @pl.when(i + 1 == n)
            def _():
                start(ffn_copies, n)

        wait(ffn_copies, i)
        r0 = pl.multiple_of(i * (NH * T), NH * T)
        v_v[:, 0:HALO, :] = v_v[:, NH * T:NH * T + HALO, :]
        first = project(i * NH, wv_v, v_v, HALO, 2)
        for j in range(NB):
            v_v[j, 0:HALO, :] = jnp.where(i > 0, v_v[j, 0:HALO, :], jnp.broadcast_to(first[j], (HALO, 128)))
        for a in range(NH):
            project(i * NH + a, wq_v, q_v, a * T, 4)
        for a in range(1, NH):
            project(i * NH + a, wv_v, v_v, HALO + a * T, 2)

        for a in range(NH):
            top, bottom = (_attend(q_v, k_v, v_v, r, r0 + r, r < HALO) for r in (a * T, a * T + M))
            for j in range(HB):
                for t, y in enumerate(_lhs_terms(top[j], top[j + HB], bottom[j], bottom[j + HB])):
                    o_v[a, t, :, 128 * j:128 * (j + 1)] = y

        for a in range(NH):
            n = D // 4
            for c0 in range(0, D // 2, n):
                y = _strassen(lambda t: o_v[a, t], lambda t: wo_v[t, :, c0:c0 + n])
                for (ra, b), c in zip(QUADRANTS, y):
                    rr, cc = pl.ds(r0 + a * T + ra * M, M), pl.ds(b * (D // 2) + c0, n)
                    h_v[rr, cc] = x_v[rr, cc].astype(f32) + c

        step = 0
        for w_ref in (wg_v, wu_v, wd_v):
            n = w_ref.shape[0] // 7 // NA
            for c in range(0, n, 16):
                for c0 in range(0, w_ref.shape[1], PC):
                    step += 1
                    _prepare_ffn(w_ref, pl.multiple_of(i * n, 16) + opaque(c, 16, i + step), c0, PC)

    normalize(h_v, 0, 0, 1)

    @pl.loop(0, NT)
    def _(i):
        for c in range(0, F // 2, FC):
            g, u = (_strassen(lambda t: n_v[i, t],
                              lambda t: _words(w_ref[t * (D // 2):(t + 1) * (D // 2), c:c + FC]))
                    for w_ref in (wg_v, wu_v))
            act = [jax.nn.gelu(a, approximate=True) * b for a, b in zip(g, u)]
            for t, a in enumerate(_lhs_terms(*act)):
                act_v[t, :, c:c + FC] = a
        for part in range(8):
            last = normalize(h_v, i + 1, part, 8)
            h_v[pl.ds(opaque(S, 8, i + 1 + part), 8), 0:128] = pltpu.bitcast(last[:, -128:], f32)
        y = _strassen(lambda t: act_v[t], lambda t: _words(wd_v[t * (F // 2):(t + 1) * (F // 2), :]), DOWN_ORDER)
        for a in (1, 0):
            rr = pl.ds(pl.multiple_of(i * T, T) + a * M, M)
            for b in (0, 1):
                cc = slice(b * (D // 2), (b + 1) * (D // 2))
                out_v[rr, cc] = (h_v[rr, cc] + y[2 * a + b]).astype(bf16)
            copy(out_v.at[rr, :], out_hbm.at[rr, :], out_sem).start()

    copy(out_v, out_hbm, out_sem).wait()


@jax.jit
def pallas_sequential_preLN__sliding_local_dilated__glu_gated_geglu__prompt_kernel(
    A_x: jax.Array,
    A_wqkv: jax.Array,
    A_wo: jax.Array,
    B_x: jax.Array,
    B_w_gate: jax.Array,
    B_w_up: jax.Array,
    B_w_down: jax.Array,
):
    del B_x
    vmem, sems = pltpu.VMEM, pltpu.SemaphoreType.DMA
    square = vmem((7, D // 4, D // 2), i32)
    any_spec = pl.BlockSpec(memory_space=pl.ANY)
    out = pl.pallas_call(
        _kernel,
        in_specs=[any_spec] * 6,
        out_specs=any_spec,
        out_shape=jax.ShapeDtypeStruct((S, D), bf16),
        scratch_shapes=[
            vmem((S, D), bf16),
            [vmem((2, D // 2, D), bf16)] * 3,
            vmem((NB, 128, D), bf16),
            vmem((7 * D // 2, F // 2), bf16),
            vmem((7 * D // 2, F // 2), bf16),
            vmem((7 * F // 2, D // 2), bf16),
            vmem((NT + 1, 7, M // 2, D // 2), i32),
            square, square, square, square,
            vmem((NB, NH * T, 128), f32),
            vmem((NB, HALO + S, 128), f32),
            vmem((NB, HALO + NH * T, 128), f32),
            vmem((NH, 7, M // 2, D // 2), i32),
            vmem((S + 8, D), f32),
            vmem((7, M // 2, F // 2), i32),
            sems((2,)), sems((4,)), sems((4,)), sems((2,)), sems(()),
        ],
        compiler_params=pltpu.CompilerParams(
            vmem_limit_bytes=120 * 1024 * 1024,
            flags={"XLA_TPU_EVENLY_DISTRIBUTE_CRITICAL_NODES": True},
        ),
    )(A_x.reshape(S, D), A_wqkv.reshape(2, D // 2, 3 * D), A_wo.reshape(NB, 128, D), B_w_gate, B_w_up, B_w_down)
    return out.reshape(1, S, D)
```
